```python
import os as _os
_os.environ.setdefault('JAX_PLATFORMS', 'cpu')
import jax
import jax.numpy as jnp

def _softmax(x, axis=-1):
    return jax.nn.softmax(x, axis=axis)

def _gelu(x):
    return jax.nn.gelu(x, approximate=True)

def _silu(x):
    return jax.nn.silu(x)

def _sigmoid(x):
    return jax.nn.sigmoid(x)

def _layernorm(x, axis=-1, eps=1e-05):
    m = jnp.mean(x, axis=axis, keepdims=True)
    v = jnp.var(x, axis=axis, keepdims=True)
    return (x - m) / jnp.sqrt(v + eps)

def _scatter_add(tgt, idx, src, axis=0):
    return tgt.at[idx].add(src)

def _segment_sum(src, seg, n):
    return jax.ops.segment_sum(src, seg, n)

class _Rng:

    def __init__(self, key):
        self._k = key

    def _next(self):
        self._k, sub = jax.random.split(self._k)
        return sub

    def normal(self, shape):
        return jax.random.normal(self._next(), shape, dtype=jnp.bfloat16)

    def randint(self, lo, hi, shape):
        return jax.random.randint(self._next(), shape, lo, hi, dtype=jnp.int32)

    def uniform(self, shape, lo=0.0, hi=1.0):
        return jax.random.uniform(self._next(), shape, jnp.bfloat16, lo, hi)

    def permutation(self, n):
        return jax.random.permutation(self._next(), n)
kernel_name = 'gated_mix__mha_block__memory_aug_recurrent_mem_tr__prompt'

def setup_inputs():
    _rng = _Rng(jax.random.key(int.from_bytes(__import__("os").urandom(4), "little")))
    _w = lambda a: (lambda t: t.astype(jnp.bfloat16) if jnp.issubdtype(t.dtype, jnp.floating) else t)(jnp.asarray(a))

    def _A_setup():
        B, S, D, H = (1, 2048, 512, 32)
        return {'x': _w((lambda *s: _rng.normal(s) * 0.05)(B, S, D)), 'wqkv': _w((lambda *s: _rng.normal(s) * 0.8)(D, 3 * D)), 'wo': _w((lambda *s: _rng.normal(s) * 0.05)(D, D))}
    _A_in = _A_setup()

    def _B_setup():
        B, S, Dm = (1, 2048, 512)
        H, Dh = (32, 128)
        M, seg = (8, 32)
        seg = min(seg, S)
        S = S // seg * seg
        return {'x': _w((lambda *s: _rng.normal(s) * 0.05)(B, S, Dm)), 'mem0': _w((lambda *s: _rng.normal(s) * 0.8)(B, M, Dm)), 'Wq': _w((lambda *s: _rng.normal(s) * 1.6)(Dm, H, Dh) * Dm ** (-0.5)), 'Wk': _w((lambda *s: _rng.normal(s) * 1.6)(Dm, H, Dh) * Dm ** (-0.5)), 'Wv': _w((lambda *s: _rng.normal(s) * 0.8)(Dm, H, Dh) * Dm ** (-0.5)), 'Wo': _w((lambda *s: _rng.normal(s) * 0.8)(H, Dh, Dm) * (H * Dh) ** (-0.5)), 'seg_len': seg}
    _B_in = _B_setup()
    return {'A_x': _A_in['x'], 'A_wqkv': _A_in['wqkv'], 'A_wo': _A_in['wo'], 'B_x': _B_in['x'], 'B_mem0': _B_in['mem0'], 'B_Wq': _B_in['Wq'], 'B_Wk': _B_in['Wk'], 'B_Wv': _B_in['Wv'], 'B_Wo': _B_in['Wo'], 'B_seg_len': _B_in['seg_len'], 'gate_w': _w((lambda *s: _rng.normal(s) * 0.05)(512) * 16.0)}

def reference(A_x, A_wqkv, A_wo, B_x, B_mem0, B_Wq, B_Wk, B_Wv, B_Wo, B_seg_len, gate_w):

    def _A_ref(x, wqkv, wo):
        B, S, D = x.shape
        H = 32
        Dh = D // H
        qkv = (lambda x, *d: x.transpose(*d))((x @ wqkv).reshape(B, S, 3, H, Dh), 2, 0, 3, 1, 4)
        q, k, v = (qkv[0], qkv[1], qkv[2])
        scores = jnp.einsum('bhqd,bhkd->bhqk', q, k) * Dh ** (-0.5)
        p = _softmax(scores, axis=-1)
        o = jnp.einsum('bhqk,bhkd->bhqd', p, v)
        return (lambda x, *d: x.transpose(*d))(o, 0, 2, 1, 3).reshape(B, S, D) @ wo

    def _B_ref(x, mem0, Wq, Wk, Wv, Wo, seg_len):
        B, S, Dm = x.shape
        H, Dh = (Wq.shape[1], Wq.shape[2])
        M = mem0.shape[1]
        scale = Dh ** (-0.5)
        n_seg = S // seg_len
        L = M + seg_len
        idx = jnp.arange(L)
        mask = (idx[:, None] < M) | (idx[:, None] >= idx[None, :])
        mem = mem0
        outs = []
        for s in range(n_seg):
            xs = x[:, s * seg_len:(s + 1) * seg_len, :].copy()
            h = jnp.concatenate([mem, xs], axis=1)
            q = jnp.einsum('btd,dhe->bhte', h, Wq)
            k = jnp.einsum('btd,dhe->bhte', h, Wk)
            v = jnp.einsum('btd,dhe->bhte', h, Wv)
            scores = jnp.einsum('bhqe,bhke->bhqk', q, k) * scale
            scores = jnp.where(mask[None, None], scores, -1000000000.0)
            p = _softmax(scores, axis=-1)
            o = jnp.einsum('bhqk,bhke->bhqe', p, v)
            o = jnp.einsum('bhte,hed->btd', o, Wo)
            mem = o[:, :M, :].copy()
            outs.append(o[:, M:, :])
        return jnp.concatenate(outs, axis=1)
    x = A_x
    g = _sigmoid((x * gate_w).sum(-1, keepdims=True))
    a = _A_ref(x, A_wqkv, A_wo)
    b = _B_ref(x, B_mem0, B_Wq, B_Wk, B_Wv, B_Wo, B_seg_len)
    return g * a + (1 - g) * b
```

```python
import functools

import jax
import jax.numpy as jnp
import numpy as np
from jax import lax
from jax.experimental import pallas as pl
from jax.experimental.pallas import tpu as pltpu

BF = jnp.bfloat16
F32 = jnp.float32

S = 2048
D = 512
HA, DHA = 32, 16
HB, DHB = 32, 128
M = 8
SEG = 32
L = M + SEG
NSEG = S // SEG
LOG2E = 1.4426950408889634

L_LO, L_HI, O_HI = 2.0 ** -30, 2.0 ** 60, 2.0 ** 120

CFG = dict(lag1=3, lag2=6, lag3=8, hb=2, kc=1024, alag=2, apos=30)


def _nt(a, b):
    return lax.dot_general(a, b, (((1,), (1,)), ((), ())), preferred_element_type=F32)


def _nn(a, b):
    return lax.dot_general(a, b, (((1,), (0,)), ((), ())), preferred_element_type=F32)


def _kernel(x_hbm, wqkv_hbm, woa_hbm, wq_hbm, wk_hbm, wv_hbm, wob_hbm, mem_ref, gate_ref,
            out_hbm,
            x_v, wqkv_v, woa_v, wraw, wob_v, w3, q_s, k_s, vt_s, ot_s, b_s, g_s, out_v,
            in_sem, out_sem, *, cfg):
    lag1, lag2, lag3 = cfg["lag1"], cfg["lag2"], cfg["lag3"]
    hb, kc, alag, apos = cfg["hb"], cfg["kc"], cfg["alag"], cfg["apos"]

    cp_x = pltpu.make_async_copy(x_hbm, x_v, in_sem.at[0])
    cp_wqkv = pltpu.make_async_copy(wqkv_hbm, wqkv_v, in_sem.at[1])
    cp_w = [pltpu.make_async_copy(src, wraw.at[i], in_sem.at[2 + i])
            for i, src in enumerate((wq_hbm, wk_hbm, wv_hbm))]
    cp_wob = pltpu.make_async_copy(wob_hbm, wob_v, in_sem.at[5])
    cp_woa = pltpu.make_async_copy(woa_hbm, woa_v, in_sem.at[6])
    cp_x.start()
    cp_wqkv.start()
    for c in cp_w:
        c.start()
    cp_wob.start()
    cp_woa.start()

    cp_wqkv.wait()
    cp_x.wait()
    qscale = DHA ** -0.5 * LOG2E
    wvt = wqkv_v[:, 2 * D:3 * D].T

    def aproj(t, c):
        rows = pl.ds(pl.multiple_of(t * 128, 128), 128)
        xb = x_v[rows, :]
        q = _nn(xb, wqkv_v[:, 0:D]) * qscale
        k = _nn(xb, wqkv_v[:, D:2 * D])
        for g in range(4):
            q_s[g, rows, :] = q[:, g * 128:(g + 1) * 128].astype(BF)
            k_s[g, rows, :] = k[:, g * 128:(g + 1) * 128].astype(BF)
        vt_s[:, rows] = _nt(wvt, xb).astype(BF)
        return c
    lax.fori_loop(0, S // 128, aproj, 0)

    for i in range(3):
        cp_w[i].wait()

        def relay(t, c, i=i):
            for u in range(2):
                r0 = pl.multiple_of((t * 2 + u) * 512, 512)
                v = wraw[i, pl.ds(r0, 512), :]
                v = jnp.swapaxes(v.reshape(16, HB, DHB), 0, 1)
                w3[:, pl.ds(pl.multiple_of((t * 2 + u) * 16, 16), 16), i * DHB:(i + 1) * DHB] = v
            return c
        lax.fori_loop(0, D // 32, relay, 0)
    cp_wob.wait()

    ri = lax.broadcasted_iota(jnp.int32, (L, L), 0)
    ci = lax.broadcasted_iota(jnp.int32, (L, L), 1)
    mask = (ri < M) | (ri >= ci)
    lane_head = lax.broadcasted_iota(jnp.int32, (128, 128), 1) // DHA
    ones128 = (lax.broadcasted_iota(jnp.int32, (16, 128), 0) == 0).astype(BF)
    ones_kc = jnp.concatenate([ones128] * (kc // 128), axis=1)
    bscale = DHB ** -0.5 * LOG2E
    gate = gate_ref[...].astype(F32).reshape(1, D)
    nch = S // kc

    def step(s, carry):
        mem, bad = carry
        st = dict(acc=None, bad=bad)
        xrows = pl.ds(pl.multiple_of(s * SEG, SEG), SEG)
        xs = x_v[xrows, :].astype(F32)
        h = jnp.concatenate([mem, xs], axis=0)
        gl = jnp.sum(xs * gate, axis=-1, keepdims=True)
        gs = 1.0 / (1.0 + jnp.exp(-gl))
        g_s[xrows, :] = jnp.broadcast_to(gs, (SEG, 128))

        qs, ks, vs, ps, os_ = {}, {}, {}, {}, {}

        def b_item(i):
            if i < HB:
                qkv = _nn(h, w3[i])
                qs[i] = qkv[:, 0:DHB]
                ks[i] = qkv[:, DHB:2 * DHB].astype(BF)
                vs[i] = qkv[:, 2 * DHB:3 * DHB].astype(BF)
            j = i - lag1
            if 0 <= j < HB:
                sc = _nt(qs.pop(j), ks.pop(j))
                t = jnp.where(mask, sc * bscale, -1e9 * LOG2E)
                m = jnp.max(t, axis=-1, keepdims=True)
                p = jnp.exp2(t - m)
                l = jnp.sum(p, axis=-1, keepdims=True)
                ps[j] = p * (1.0 / l)
            j = i - lag2
            if 0 <= j < HB:
                os_[j] = _nn(ps.pop(j), vs.pop(j))
            j = i - lag3
            if 0 <= j < HB:
                r = _nn(os_.pop(j), wob_v[j * DHB:(j + 1) * DHB, :])
                st["acc"] = r if st["acc"] is None else st["acc"] + r

        g = s % 4
        qt = s // 4
        qcols = pl.ds(pl.multiple_of(qt * 128, 128), 128)
        work = [(b, ch) for b in range(0, 8, hb) for ch in range(nch)]
        pts, accs = {}, {}

        def a_item(i):
            if i < len(work):
                b, ch = work[i]
                qv = q_s[g, qcols, :]
                qm = jnp.concatenate(
                    [jnp.where(lane_head == b + u, qv, jnp.zeros_like(qv)) for u in range(hb)], axis=0)
                sT = _nt(k_s[g, ch * kc:(ch + 1) * kc, :], qm)
                pts[i] = jnp.exp2(sT).astype(BF)
            j = i - alag
            if j >= 0:
                b, ch = work[j]
                pj = pts.pop(j)
                for u in range(hb):
                    hrow = pl.ds(pl.multiple_of(g * 128 + (b + u) * DHA, DHA), DHA)
                    lhs = jnp.concatenate([vt_s[hrow, ch * kc:(ch + 1) * kc], ones_kc], axis=0)
                    r = _nn(lhs, pj[:, u * 128:(u + 1) * 128])
                    accs[b + u] = r if ch == 0 else accs[b + u] + r
                    if ch == nch - 1:
                        o = accs.pop(b + u)
                        l = o[DHA:DHA + 1, :]
                        ov = o[0:DHA, :]
                        ot_s[hrow, qcols] = (ov * (1.0 / l)).astype(BF)
                        ok = (l >= L_LO) & (l <= L_HI)
                        ok2 = jnp.abs(ov) < O_HI
                        st["bad"] = jnp.maximum(st["bad"], jnp.maximum(
                            jnp.where(ok, 0.0, 1.0), jnp.where(ok2, 0.0, 1.0)[0:8] + jnp.where(ok2, 0.0, 1.0)[8:16]))

        nb_items = HB + lag3
        na_items = len(work) + alag
        for i in range(apos):
            b_item(i)
        rest = nb_items - apos
        ai = 0
        for bi in range(rest):
            while ai < na_items and ai * rest <= bi * na_items:
                a_item(ai)
                ai += 1
            b_item(apos + bi)
        while ai < na_items:
            a_item(ai)
            ai += 1

        out = st["acc"]
        b_s[xrows, :] = out[M:, :] * (1.0 - gs)
        return out[:M, :], st["bad"]

    _, bad = lax.fori_loop(0, NSEG, step, (mem_ref[...].astype(F32), jnp.zeros((8, 128), F32)))

    @pl.when(jnp.max(bad) > 0.0)
    def _():
        def safe_block(i, c):
            hh = i // (S // 128)
            qt = i % (S // 128)
            g = hh // 8
            qcols = pl.ds(pl.multiple_of(qt * 128, 128), 128)
            hrow = pl.ds(pl.multiple_of(hh * DHA, DHA), DHA)
            qv = q_s[g, qcols, :]
            qm = jnp.where(lane_head == hh % 8, qv, jnp.zeros_like(qv))
            ck = 256

            def pass1(ch, m):
                sT = _nt(k_s[g, pl.ds(pl.multiple_of(ch * ck, ck), ck), :], qm)
                return jnp.maximum(m, jnp.max(sT, axis=0, keepdims=True))
            m = lax.fori_loop(0, S // ck, pass1, jnp.full((1, 128), -jnp.inf, F32))

            def pass2(ch, o):
                kr = pl.ds(pl.multiple_of(ch * ck, ck), ck)
                sT = _nt(k_s[g, kr, :], qm)
                p = jnp.exp2(sT - m).astype(BF)
                lhs = jnp.concatenate([vt_s[hrow, kr], jnp.concatenate([ones128] * (ck // 128), axis=1)], axis=0)
                return o + _nn(lhs, p)
            o = lax.fori_loop(0, S // ck, pass2, jnp.zeros((2 * DHA, 128), F32))
            ot_s[hrow, qcols] = (o[0:DHA, :] * (1.0 / o[DHA:DHA + 1, :])).astype(BF)
            return c
        lax.fori_loop(0, HA * (S // 128), safe_block, 0)

    cp_woa.wait()

    def out_copy(t):
        rows = pl.ds(pl.multiple_of(t * 128, 128), 128)
        return pltpu.make_async_copy(out_v.at[rows, :], out_hbm.at[rows, :], out_sem.at[t])

    def final(t, c):
        rows = pl.ds(pl.multiple_of(t * 128, 128), 128)
        a = lax.dot_general(ot_s[:, rows], woa_v[...], (((0,), (0,)), ((), ())), preferred_element_type=F32)
        gq = g_s[rows, :]
        gq4 = jnp.concatenate([gq] * (D // 128), axis=1)
        out_v[rows, :] = (gq4 * a + b_s[rows, :]).astype(BF)
        out_copy(t).start()
        return c
    lax.fori_loop(0, S // 128, final, 0)

    def drain(t, c):
        out_copy(t).wait()
        return c
    lax.fori_loop(0, S // 128, drain, 0)


@functools.partial(jax.jit, static_argnames=("cfg",))
def _impl(A_x, A_wqkv, A_wo, B_mem0, B_Wq, B_Wk, B_Wv, B_Wo, gate_w, cfg=None):
    cfg = dict(CFG if cfg is None else dict(cfg))
    any_spec = pl.BlockSpec(memory_space=pl.ANY)
    vmem_spec = pl.BlockSpec(memory_space=pltpu.VMEM)
    out = pl.pallas_call(
        functools.partial(_kernel, cfg=cfg),
        out_shape=jax.ShapeDtypeStruct((S, D), BF),
        in_specs=[any_spec] * 7 + [vmem_spec, vmem_spec],
        out_specs=any_spec,
        scratch_shapes=[
            pltpu.VMEM((S, D), BF),
            pltpu.VMEM((D, 3 * D), BF),
            pltpu.VMEM((D, D), BF),
            pltpu.VMEM((3, D * HB, DHB), BF),
            pltpu.VMEM((HB * DHB, D), BF),
            pltpu.VMEM((HB, D, 3 * DHB), BF),
            pltpu.VMEM((4, S, 128), BF),
            pltpu.VMEM((4, S, 128), BF),
            pltpu.VMEM((D, S), BF),
            pltpu.VMEM((D, S), BF),
            pltpu.VMEM((S, D), F32),
            pltpu.VMEM((S, 128), F32),
            pltpu.VMEM((S, D), BF),
            pltpu.SemaphoreType.DMA((7,)),
            pltpu.SemaphoreType.DMA((S // 128,)),
        ],
        compiler_params=pltpu.CompilerParams(vmem_limit_bytes=100 * 2 ** 20),
        name="gated_mix_kernel",
    )(A_x.reshape(S, D), A_wqkv, A_wo,
      B_Wq.reshape(D * HB, DHB), B_Wk.reshape(D * HB, DHB), B_Wv.reshape(D * HB, DHB),
      B_Wo.reshape(HB * DHB, D), B_mem0.reshape(M, D), gate_w)
    return out.reshape(1, S, D)


def pallas_gated_mix__mha_block__memory_aug_recurrent_mem_tr__prompt_kernel(
    A_x, A_wqkv, A_wo, B_x, B_mem0, B_Wq, B_Wk, B_Wv, B_Wo, B_seg_len, gate_w,
):
    del B_x
    if isinstance(B_seg_len, int):
        assert B_seg_len == SEG, "kernel is specialised to seg_len == 32"
    return _impl(A_x, A_wqkv, A_wo, B_mem0, B_Wq, B_Wk, B_Wv, B_Wo, gate_w)
```

```python
import contextlib
import functools

import jax
import jax.numpy as jnp
import numpy as np
from jax import lax
from jax.experimental import pallas as pl
from jax.experimental.pallas import tpu as pltpu

BF = jnp.bfloat16
F32 = jnp.float32
U32 = jnp.uint32

S = 2048
D = 512
HA, DHA = 32, 16
HB, DHB = 32, 128
M = 8
SEG = 32
L = M + SEG
NSEG = S // SEG
LOG2E = 1.4426950408889634

L_LO, L_HI, O_HI = 2.0 ** -30, 2.0 ** 60, 2.0 ** 120

CFG = dict(lag1=4, lag2=8, lag3=16, hb=4, kc=128, alag=2, mode="apos", apos=0, aend=0, astart=0.0, astop=1.0, order="hc", unroll=2, wdef=8, wdyn=0, look=4, wob_at=14, fun=4, xch=4, scopes=0, wou=1, dma="staged", pw=1, po=1, npre=2, relay_in_pre=1, lead=0.0, ramp=0.5, qT=1, relay_split=8, aun=2, merge_final=1, late_pos=0.4)


def _nt(a, b):
    return lax.dot_general(a, b, (((1,), (1,)), ((), ())), preferred_element_type=F32)


def _nn(a, b):
    return lax.dot_general(a, b, (((1,), (0,)), ((), ())), preferred_element_type=F32)


def _kernel(x_hbm, wqkv_hbm, woa_hbm, wq_hbm, wk_hbm, wv_hbm, wob_hbm, mem_ref, gate_ref,
            out_hbm,
            x_v, wqkv_v, woa_v, wraw, wob_v, w3, q_s, k_s, vt_s, ot_s, b_s, g_s, out_v,
            o_buf, wvt_s, in_sem, x_sem, w_sem, out_sem, *, cfg):
    lag1, lag2, lag3 = cfg["lag1"], cfg["lag2"], cfg["lag3"]
    hb, kc, alag = cfg["hb"], cfg["kc"], cfg["alag"]

    xch = cfg["xch"]
    scope = (lambda n: jax.named_scope(n)) if cfg["scopes"] else (lambda n: contextlib.nullcontext())
    xr = S // xch
    NW = HB // 2
    w_src = tuple(w.bitcast(U32) for w in (wq_hbm, wk_hbm, wv_hbm))

    def cp_x(c):
        return pltpu.make_async_copy(x_hbm.at[c * xr:(c + 1) * xr, :], x_v.at[c * xr:(c + 1) * xr, :], x_sem.at[c])

    def cp_w(j, i):
        return pltpu.make_async_copy(w_src[i].at[:, j, :], wraw.at[i, j], w_sem.at[j * 3 + i])

    cp_wqkv = pltpu.make_async_copy(wqkv_hbm, wqkv_v, in_sem.at[0])
    cp_wob = pltpu.make_async_copy(wob_hbm.bitcast(U32) if cfg["wou"] else wob_hbm, wob_v, in_sem.at[1])
    cp_woa = pltpu.make_async_copy(woa_hbm, woa_v, in_sem.at[2])
    look, wob_at = cfg["look"], cfg["wob_at"]
    NT = S // 128
    tpx = NT // xch

    dma = cfg["dma"]
    if dma == "staged":
        cp_wqkv.start()
        cp_x(0).start()
        with scope("ph_0_wait_wqkv"):
            cp_wqkv.wait()
            cp_x(0).wait()
        for w in range(look):
            for i in range(3):
                cp_w(w, i).start(priority=cfg["pw"])
    else:
        cp_wqkv.start()
        for c in range(xch):
            cp_x(c).start()
        for w in range(NW):
            for i in range(3):
                cp_w(w, i).start(priority=cfg["pw"])
        cp_wob.start(priority=cfg["po"])
        cp_woa.start(priority=cfg["po"])
        with scope("ph_0_wait_wqkv"):
            cp_wqkv.wait()
            cp_x(0).wait()

    qt_ref = q_s

    qscale = DHA ** -0.5 * LOG2E
    qT = cfg["qT"]
    wvt_s[0] = wqkv_v[:, 2 * D:3 * D].T
    if qT:
        wvt_s[1] = wqkv_v[:, 0:D].T

    def relay(j, i):
        cols = slice(i * DHB, (i + 1) * DHB)
        for u in range(4):
            ev = wraw[i, j, pl.ds(u * 128, 64, stride=2), :]
            od = wraw[i, j, pl.ds(u * 128 + 1, 64, stride=2), :]
            rows = slice(u * 64, (u + 1) * 64)
            w3[2 * j, rows, cols] = (ev & np.uint32(0xFFFF)) | (od << 16)
            w3[2 * j + 1, rows, cols] = (ev >> 16) | (od & np.uint32(0xFFFF0000))

    def aproj(t):
        rows = pl.ds(pl.multiple_of(t * 128, 128), 128)
        xb = x_v[rows, :]
        if qT:
            qt_ref[:, rows] = (_nt(wvt_s[1], xb) * qscale).astype(BF)
        else:
            q = _nn(xb, wqkv_v[:, 0:D]) * qscale
            for g in range(4):
                q_s[g, rows, :] = q[:, g * 128:(g + 1) * 128].astype(BF)
        k = _nn(xb, wqkv_v[:, D:2 * D])
        for g in range(4):
            k_s[g, rows, :] = k[:, g * 128:(g + 1) * 128].astype(BF)
        vt_s[:, rows] = _nt(wvt_s[0], xb).astype(BF)

    def wait_w(c):
        for i in range(3):
            cp_w(c, i).wait()

    def start_w(c):
        for i in range(3):
            cp_w(c, i).start(priority=cfg["pw"])

    aun = cfg["aun"]
    extra = {}
    if dma == "staged":
        for c in range(1, xch):
            extra.setdefault((c - 1) * tpx, []).append((cp_x(c), 0))
    else:
        look = NW
    last_start = -((look - NW) // aun) * aun
    cuts = sorted({0, NT, last_start} | set(extra) | {c * tpx for c in range(xch)})
    started = look
    for lo, hi in zip(cuts[:-1], cuts[1:]):
        assert lo % aun == 0 and hi % aun == 0
        if lo % tpx == 0 and lo > 0:
            with scope("ph_1_wait_x"):
                cp_x(lo // tpx).wait()
        for cp, pr in extra.get(lo, []):
            cp.start(priority=pr)
        n_start = 0
        if lo < last_start:
            n_start = aun
            total = (hi - lo) // aun * n_start
            if started + total > NW:
                for j in range(started, NW):
                    start_w(j)
                started, n_start = NW, 0
        first = started

        def body_p(t, carry, n_start=n_start, first=first, lo=lo):
            for k in range(n_start):
                start_w(first + (t - lo // aun) * n_start + k)
            for u in range(aun):
                aproj(t * aun + u)
            return carry
        with scope("ph_3_aproj"):
            lax.fori_loop(lo // aun, hi // aun, body_p, 0)
        started += (hi - lo) // aun * n_start
    for j in range(started, NW):
        start_w(j)

    split = cfg["relay_split"] if (cfg["npre"] == 2 and cfg["relay_in_pre"]) else NW

    def wait_all_w(j, c):
        wait_w(j)
        return c
    with scope("ph_3w_wait_w"):
        lax.fori_loop(0, split, wait_all_w, 0)

    def late_dmas():
        for j in range(split, NW):
            wait_w(j)
        if dma == "staged":
            cp_wob.start(priority=cfg["po"])
            cp_woa.start(priority=cfg["po"])
    if split == NW:
        late_dmas()

    ri = lax.broadcasted_iota(jnp.int32, (L, L), 0)
    ci = lax.broadcasted_iota(jnp.int32, (L, L), 1)
    mask = (ri < M) | (ri >= ci)
    lane_head = lax.broadcasted_iota(jnp.int32, (128, 128), 1) // DHA
    row_head = lax.broadcasted_iota(jnp.int32, (128, 128), 0) // DHA
    ones128 = (lax.broadcasted_iota(jnp.int32, (16, 128), 0) == 0).astype(BF)
    bscale = DHB ** -0.5 * LOG2E
    gate = gate_ref[...].astype(F32).reshape(1, D)
    nch = S // kc

    wdef = cfg["wdef"]
    nb_items = max(HB - wdef + lag3, HB + lag2 + (wdef + 3) // 4) if wdef else HB + lag3

    def b_stream(s, box):
        loc = dict(acc=None)
        qs, ks, vs, ps, os_ = {}, {}, {}, {}, {}
        xrows = pl.ds(pl.multiple_of(s * SEG, SEG), SEG)

        def init():
            xs = x_v[xrows, :].astype(F32)
            loc["h"] = jnp.concatenate([box["mem"], xs], axis=0)
            gl = jnp.sum(xs * gate, axis=-1, keepdims=True)
            loc["gs"] = 1.0 / (1.0 + jnp.exp(-gl))
            g_s[xrows, :] = jnp.broadcast_to(loc["gs"], (SEG, 128))

        def wo_item(j, o):
            wo_j = pltpu.bitcast(wob_v[j * 64:(j + 1) * 64, :], BF) if cfg["wou"] else wob_v[j * DHB:(j + 1) * DHB, :]
            r = _nn(o, wo_j)
            loc["acc"] = r if loc["acc"] is None else loc["acc"] + r

        def item(i):
            if i == 0:
                init()
            if i < HB:
                qkv = _nn(loc["h"], pltpu.bitcast(w3[i], BF))
                qs[i] = qkv[:, 0:DHB]
                ks[i] = qkv[:, DHB:2 * DHB].astype(BF)
                vs[i] = qkv[:, 2 * DHB:3 * DHB].astype(BF)
            j = i - lag1
            if 0 <= j < HB:
                sc = _nt(qs.pop(j), ks.pop(j))
                t = jnp.where(mask, sc * bscale, -1e9 * LOG2E)
                m = jnp.max(t, axis=-1, keepdims=True)
                p = jnp.exp2(t - m)
                l = jnp.sum(p, axis=-1, keepdims=True)
                ps[j] = p * (1.0 / l)
            j = i - lag2
            if 0 <= j < HB:
                o = _nn(ps.pop(j), vs.pop(j))
                if j >= HB - wdef:
                    o_buf[j - (HB - wdef)] = o
                else:
                    os_[j] = o
            j = i - lag3
            if 0 <= j < HB - wdef:
                wo_item(j, os_.pop(j))
            if wdef and i >= HB - 1 + lag2:
                k0 = i - (HB - 1 + lag2)
                n_left = nb_items - (HB - 1 + lag2)
                for jj in range(k0 * wdef // n_left, (k0 + 1) * wdef // n_left):
                    wo_item(HB - wdef + jj, o_buf[jj])
            if i == nb_items - 1:
                out = loc["acc"]
                b_s[xrows, :] = out[M:, :] * (1.0 - loc["gs"])
                box["mem"] = out[:M, :]
        return [functools.partial(item, i) for i in range(nb_items)]

    if cfg["order"] == "hc":
        work = [(b, ch) for b in range(0, 8, hb) for ch in range(nch)]
    else:
        work = [(b, ch) for ch in range(nch) for b in range(0, 8, hb)]
    na_items = len(work) + alag

    qk = _nn if qT else _nt

    def masked_q(g, qcols, hh):
        if not qT:
            qv = q_s[g, qcols, :]
            return jnp.where(lane_head == hh, qv, jnp.zeros_like(qv))
        if isinstance(hh, int):
            qh = qt_ref[pl.ds(pl.multiple_of(g * 128 + hh * DHA, DHA), DHA), qcols]
            z = jnp.zeros((DHA, 128), BF)
            return jnp.concatenate([z] * hh + [qh] + [z] * (7 - hh), axis=0)
        qv = qt_ref[pl.ds(pl.multiple_of(g * 128, 128), 128), qcols]
        return jnp.where(row_head == hh, qv, jnp.zeros_like(qv))

    def a_stream(sa, box):
        g, qt = sa % 4, sa // 4
        qcols = pl.ds(pl.multiple_of(qt * 128, 128), 128)
        pts, accs, ls, qms = {}, {}, {}, {}

        def item(i):
            if i == 0:
                for b in range(0, 8, hb):
                    qms[b] = jnp.concatenate([masked_q(g, qcols, b + u) for u in range(hb)], axis=1 if qT else 0)
            if i < len(work):
                b, ch = work[i]
                sT = qk(k_s[g, ch * kc:(ch + 1) * kc, :], qms[b])
                p = jnp.exp2(sT)
                lp = p[0:8]
                for r in range(1, kc // 8):
                    lp = lp + p[8 * r:8 * r + 8]
                ls[b] = lp if ch == 0 else ls[b] + lp
                pts[i] = p.astype(BF)
            j = i - alag
            if j >= 0:
                b, ch = work[j]
                pj = pts.pop(j)
                for u in range(hb):
                    hrow = pl.ds(pl.multiple_of(g * 128 + (b + u) * DHA, DHA), DHA)
                    r = _nn(vt_s[hrow, ch * kc:(ch + 1) * kc], pj[:, u * 128:(u + 1) * 128])
                    accs[b + u] = r if ch == 0 else accs[b + u] + r
                    if ch == nch - 1:
                        o = accs.pop(b + u)
                        l = jnp.sum(ls[b][:, u * 128:(u + 1) * 128], axis=0, keepdims=True)
                        ot_s[hrow, qcols] = (o * (1.0 / l)).astype(BF)
                        ok = (l >= L_LO) & (l <= L_HI)
                        bad_o = jnp.where(jnp.abs(o) < O_HI, 0.0, 1.0)
                        box["bad"] = jnp.maximum(box["bad"], jnp.maximum(
                            jnp.where(ok, 0.0, 1.0), jnp.maximum(bad_o[0:8], bad_o[8:16])))
        return [functools.partial(item, i) for i in range(na_items)]

    def run_streams(first, second, lead=0.0, flat=0):
        nf, ns = len(first), len(second)
        si = 0
        for fi in range(nf):
            x = fi / nf
            if flat:
                target = x * ns
            else:
                pos = x * nun
                edge = min(pos, nun - pos, ramp) / ramp if ramp > 0 else 0.0
                target = (pos + lead * edge) / nun * ns
            while si < ns and si <= target:
                second[si]()
                si += 1
            first[fi]()
        while si < ns:
            second[si]()
            si += 1

    def body(sb_list, sa_list, carry, fill=None):
        box = dict(mem=carry[0], bad=carry[1])
        bs = [it for sb in sb_list for it in b_stream(sb, box)]
        as_ = [it for sa in sa_list for it in a_stream(sa, box)]
        if bs and as_:
            run_streams(bs, as_, cfg["lead"])
        elif bs:
            run_streams(bs, fill or [], flat=1)
        else:
            run_streams(as_, fill or [], flat=1)
        return box["mem"], box["bad"]

    un, npre = cfg["unroll"], cfg["npre"]
    nun, ramp = un, cfg["ramp"]
    carry = (mem_ref[...].astype(F32), jnp.zeros((8, 128), F32))

    def relay_all():
        def body_r(j, c):
            for i in range(3):
                relay(j, i)
            return c
        lax.fori_loop(0, NW, body_r, 0)

    if npre:
        with scope("ph_4a_pre"):
            if cfg["relay_in_pre"]:
                bounds = (0, cfg["relay_split"], NW) if npre == 2 else (0,) * npre + (NW,)
                for t in range(npre):
                    lo_, hi_ = bounds[t], bounds[t + 1]
                    fill = [functools.partial(relay, j, i) for j in range(lo_, hi_) for i in range(3)]
                    if t == 0 and split < NW:
                        fill.insert(int(cfg["late_pos"] * len(fill)), late_dmas)
                    with scope("ph_4x%d" % t):
                        carry = body([], [t], carry, fill)
            else:
                carry = lax.fori_loop(0, npre, lambda t, c: body([], [t], c), carry)
    if not (npre and cfg["relay_in_pre"]):
        with scope("ph_4_relay"):
            relay_all()
    with scope("ph_5_wait_wob"):
        cp_wob.wait()

    def step_u(t, c):
        return body([t * un + u for u in range(un)], [t * un + u + npre for u in range(un)], c)

    assert (NSEG - npre) % un == 0
    with scope("ph_6_main"):
        carry = lax.fori_loop(0, (NSEG - npre) // un, step_u, carry)
    @pl.when(jnp.max(carry[1]) > 0.0)
    def _():
        def safe_block(i, c):
            hh = i // (S // 128)
            qt = i % (S // 128)
            g = hh // 8
            qcols = pl.ds(pl.multiple_of(qt * 128, 128), 128)
            hrow = pl.ds(pl.multiple_of(hh * DHA, DHA), DHA)
            qm = masked_q(g, qcols, hh % 8)
            ck = 256

            def pass1(ch, m):
                sT = qk(k_s[g, pl.ds(pl.multiple_of(ch * ck, ck), ck), :], qm)
                return jnp.maximum(m, jnp.max(sT, axis=0, keepdims=True))
            m = lax.fori_loop(0, S // ck, pass1, jnp.full((1, 128), -jnp.inf, F32))

            def pass2(ch, o):
                kr = pl.ds(pl.multiple_of(ch * ck, ck), ck)
                sT = qk(k_s[g, kr, :], qm)
                p = jnp.exp2(sT - m).astype(BF)
                lhs = jnp.concatenate([vt_s[hrow, kr], jnp.concatenate([ones128] * (ck // 128), axis=1)], axis=0)
                return o + _nn(lhs, p)
            o = lax.fori_loop(0, S // ck, pass2, jnp.zeros((2 * DHA, 128), F32))
            ot_s[hrow, qcols] = (o[0:DHA, :] * (1.0 / o[DHA:DHA + 1, :])).astype(BF)
            return c
        lax.fori_loop(0, HA * (S // 128), safe_block, 0)

    cp_woa.wait()

    def out_copy(t):
        rows = pl.ds(pl.multiple_of(t * 128, 128), 128)
        return pltpu.make_async_copy(out_v.at[rows, :], out_hbm.at[rows, :], out_sem.at[t])

    def final_tile(t):
        rows = pl.ds(pl.multiple_of(t * 128, 128), 128)
        a = _nn(ot_s[:, rows].T, woa_v[...])
        gq = g_s[rows, :]
        gq4 = jnp.concatenate([gq] * (D // 128), axis=1)
        out_v[rows, :] = (gq4 * a + b_s[rows, :]).astype(BF)
        out_copy(t).start()

    NQ = S // 128
    if npre and cfg["merge_final"]:
        ready = (NSEG - npre) * SEG // 128
        with scope("ph_6b_post"):
            for k in range(npre):
                tiles = range(k * ready // npre, (k + 1) * ready // npre)
                carry = body([NSEG - npre + k], [], carry, [functools.partial(final_tile, t) for t in tiles])
        with scope("ph_7_final"):
            for t in range(ready, NQ):
                final_tile(t)
    else:
        if npre:
            with scope("ph_6b_post"):
                carry = lax.fori_loop(NSEG - npre, NSEG, lambda t, c: body([t], [], c), carry)
        fun = cfg["fun"]

        def final(tt, c):
            for u in range(fun):
                final_tile(tt * fun + u)
            return c
        with scope("ph_7_final"):
            lax.fori_loop(0, NQ // fun, final, 0)

    def drain(t, c):
        out_copy(t).wait()
        return c
    with scope("ph_8_drain"):
        lax.fori_loop(0, NQ, drain, 0)


@functools.partial(jax.jit, static_argnames=("cfg",))
def _impl(A_x, A_wqkv, A_wo, B_mem0, B_Wq, B_Wk, B_Wv, B_Wo, gate_w, cfg=None):
    cfg = dict(CFG if cfg is None else dict(cfg))
    any_spec = pl.BlockSpec(memory_space=pl.ANY)
    vmem_spec = pl.BlockSpec(memory_space=pltpu.VMEM)
    out = pl.pallas_call(
        functools.partial(_kernel, cfg=cfg),
        out_shape=jax.ShapeDtypeStruct((S, D), BF),
        in_specs=[any_spec] * 7 + [vmem_spec, vmem_spec],
        out_specs=any_spec,
        scratch_shapes=[
            pltpu.VMEM((S, D), BF),
            pltpu.VMEM((D, 3 * D), BF),
            pltpu.VMEM((D, D), BF),
            pltpu.VMEM((3, HB // 2, D, DHB), U32),
            pltpu.VMEM((HB * DHB // 2, D), U32) if cfg["wou"] else pltpu.VMEM((HB * DHB, D), BF),
            pltpu.VMEM((HB, D // 2, 3 * DHB), U32),
            pltpu.VMEM((D, S), BF) if cfg["qT"] else pltpu.VMEM((4, S, 128), BF),
            pltpu.VMEM((4, S, 128), BF),
            pltpu.VMEM((D, S), BF),
            pltpu.VMEM((D, S), BF),
            pltpu.VMEM((S, D), F32),
            pltpu.VMEM((S, 128), F32),
            pltpu.VMEM((S, D), BF),
            pltpu.VMEM((max(cfg["wdef"], 1), L, DHB), F32),
            pltpu.VMEM((2, D, D), BF),
            pltpu.SemaphoreType.DMA((3,)),
            pltpu.SemaphoreType.DMA((cfg["xch"],)),
            pltpu.SemaphoreType.DMA((48,)),
            pltpu.SemaphoreType.DMA((S // 128,)),
        ],
        compiler_params=pltpu.CompilerParams(vmem_limit_bytes=100 * 2 ** 20),
        name="gated_mix_kernel",
    )(A_x.reshape(S, D), A_wqkv, A_wo,
      B_Wq, B_Wk, B_Wv,
      B_Wo.reshape(HB * DHB, D), B_mem0.reshape(M, D), gate_w)
    return out.reshape(1, S, D)


def pallas_gated_mix__mha_block__memory_aug_recurrent_mem_tr__prompt_kernel(
    A_x, A_wqkv, A_wo, B_x, B_mem0, B_Wq, B_Wk, B_Wv, B_Wo, B_seg_len, gate_w,
):
    del B_x
    if isinstance(B_seg_len, int):
        assert B_seg_len == SEG, "kernel is specialised to seg_len == 32"
    return _impl(A_x, A_wqkv, A_wo, B_mem0, B_Wq, B_Wk, B_Wv, B_Wo, gate_w)
```

```python
import contextlib
import functools

import jax
import jax.numpy as jnp
import numpy as np
from jax import lax
from jax.experimental import pallas as pl
from jax.experimental.pallas import tpu as pltpu

BF = jnp.bfloat16
F32 = jnp.float32
U32 = jnp.uint32

S = 2048
D = 512
HA, DHA = 32, 16
HB, DHB = 32, 128
M = 8
SEG = 32
L = M + SEG
NSEG = S // SEG
NQ = S // 128
NW = 16
LOG2E = 1.4426950408889634
LO16, HI16 = np.uint32(0x0000FFFF), np.uint32(0xFFFF0000)

L_LO, L_HI, O_HI = 2.0 ** -30, 2.0 ** 60, 2.0 ** 120

CFG = dict(lag1=4, lag2=8, lag3=16, wdef=8, alag=2, order="hc", unroll=2, npre=2,
           aun=2, look=4, rlag=4, wob_at=-1, fsplit=10, pw=1, po=1, lead=0.0, ramp=0.5, scopes=0, pieces="par")


def _nt(a, b):
    return lax.dot_general(a, b, (((1,), (1,)), ((), ())), preferred_element_type=F32)


def _nn(a, b):
    return lax.dot_general(a, b, (((1,), (0,)), ((), ())), preferred_element_type=F32)


def _pack(v):
    return pltpu.bitcast(v, U32)


def _unpack(v):
    return pltpu.bitcast(v, BF)


def _ds(start, size):
    if isinstance(start, int):
        return pl.ds(start, size)
    return pl.ds(pl.multiple_of(start, size), size)


def _dma_block(n, fn):
    if isinstance(n, int) and n <= 0:
        return

    def body(k, c):
        fn(k)
        return c
    lax.fori_loop(0, n, body, 0)


def _interleave(first, second):
    nf, ns = len(first), len(second)
    si = 0
    for fi in range(nf):
        while si < ns and si * nf <= fi * ns:
            second[si]()
            si += 1
        first[fi]()
    while si < ns:
        second[si]()
        si += 1


def _kernel(x_hbm, wqkv_hbm, woa_hbm, wq_hbm, wk_hbm, wv_hbm, wob_hbm, mem_ref, gate_ref,
            out_hbm,
            x_v, wqkv_v, woa_v, wraw, wob_v, xu, wtu, wku, w3, qt_u, k_u, vt_u, ot_s, b_s, g_s,
            out_v, o_buf, in_sem, x_sem, w_sem, out_sem, *, cfg):
    lag1, lag2, lag3, wdef, alag = cfg["lag1"], cfg["lag2"], cfg["lag3"], cfg["wdef"], cfg["alag"]
    un, npre, aun, look, rlag = cfg["unroll"], cfg["npre"], cfg["aun"], cfg["look"], cfg["rlag"]
    scope = jax.named_scope if cfg["scopes"] else (lambda n: contextlib.nullcontext())
    xch = 4
    xr = S // xch

    w_src = (wq_hbm, wk_hbm, wv_hbm)
    wr = (D // NW) * HB

    def cp_x(c):
        return pltpu.make_async_copy(x_hbm.at[pl.ds(c * xr, xr), :], x_v.at[pl.ds(c * xr, xr), :], x_sem.at[c])

    def cp_w(j, i):
        rows = _ds(j * wr, wr)
        return pltpu.make_async_copy(w_src[i].at[rows, :], wraw.at[i, rows, :], w_sem.at[j * 3 + i])

    def start_w(j):
        for i in range(3):
            cp_w(j, i).start(priority=cfg["pw"])

    def wait_w(j):
        for i in range(3):
            cp_w(j, i).wait()

    cp_wqkv = pltpu.make_async_copy(wqkv_hbm, wqkv_v, in_sem.at[0])
    cp_wob = pltpu.make_async_copy(wob_hbm, wob_v, in_sem.at[1])
    cp_woa = pltpu.make_async_copy(woa_hbm, woa_v, in_sem.at[2])

    def cp_out(t):
        rows = _ds(t * 128, 128)
        return pltpu.make_async_copy(out_v.at[rows, :], out_hbm.at[rows, :], out_sem.at[t])

    def start_late():
        cp_wob.start(priority=cfg["po"])
        cp_woa.start(priority=cfg["po"])

    cp_wqkv.start()
    cp_x(0).start()
    with scope("ph_0_wait"):
        cp_wqkv.wait()
        cp_x(0).wait()
    for j in range(look):
        start_w(j)

    sub_id = lax.broadcasted_iota(jnp.int32, (8, 128), 0)

    def transpose8(vs):
        for dist in (4, 2, 1):
            keep = (sub_id & dist) == 0
            new = list(vs)
            for a in range(8):
                if a & dist == 0:
                    x, y = vs[a], vs[a + dist]
                    new[a] = jnp.where(keep, x, pltpu.roll(y, dist, 0))
                    new[a + dist] = jnp.where(keep, pltpu.roll(x, 8 - dist, 0), y)
            vs = new
        return vs

    def relay_piece(j, i, u, half, par):
        blk = j * 2 + u
        r0 = (blk * 512 if isinstance(blk, int) else pl.multiple_of(blk * 512, 512)) + 16 * half
        lst = []
        for r in range(8):
            w0 = _pack(wraw[i, pl.ds(r0 + (2 * r) * HB, 16), :])
            w1 = _pack(wraw[i, pl.ds(r0 + (2 * r + 1) * HB, 16), :])
            lst.append((w0 & LO16) | (w1 << 16) if par == 0 else (w0 >> 16) | (w1 & HI16))
        lst = transpose8(lst)
        for p in range(8):
            w3[16 * half + 2 * p + par, _ds(blk * 8, 8), i * DHB:(i + 1) * DHB] = lst[p]

    def relay_pieces(j):
        return [functools.partial(relay_piece, j, i, u, half, par)
                for i in range(3) for u in range(2) for half in range(2) for par in range(2)]

    qscale = DHA ** -0.5 * LOG2E
    wtu[0] = _pack(wqkv_v[:, 0:D].T)
    wtu[1] = _pack(wqkv_v[:, 2 * D:3 * D].T)
    wku[...] = _pack(wqkv_v[:, D:2 * D])

    def pack_x(c):
        def body(t, carry):
            xu[_ds(c * (xr // 2) + t * 64, 64), :] = _pack(x_v[_ds(c * xr + t * 128, 128), :])
            return carry
        lax.fori_loop(0, xr // 128, body, 0)

    def aproj_items(t):
        cols = _ds(t * 128, 128)
        st = {}

        def xb():
            if "x" not in st:
                st["x"] = _unpack(xu[_ds(t * 64, 64), :])
            return st["x"]

        def qt(g):
            r = _nt(_unpack(wtu[0, g * 64:(g + 1) * 64, :]), xb()) * qscale
            qt_u[g * 64:(g + 1) * 64, cols] = _pack(r.astype(BF))

        def kk(g):
            r = _nn(xb(), _unpack(wku[:, g * 128:(g + 1) * 128]))
            k_u[g, _ds(t * 64, 64), :] = _pack(r.astype(BF))

        def vt(g):
            r = _nt(_unpack(wtu[1, g * 64:(g + 1) * 64, :]), xb())
            vt_u[g * 64:(g + 1) * 64, cols] = _pack(r.astype(BF))
        return [functools.partial(f, g) for f in (kk, qt, vt) for g in range(4)]

    nit = NQ // aun
    ipx = nit // xch
    assert (NW - look) % aun == 0 and rlag % aun == 0
    last_start = (NW - look) // aun
    wob_it = cfg["wob_at"]
    cuts = sorted({0, nit, rlag // aun, last_start} | {c * ipx for c in range(xch)} | ({wob_it} if wob_it >= 0 else set()))
    for lo, hi in zip(cuts[:-1], cuts[1:]):
        if lo % ipx == 0:
            c = lo // ipx
            if c > 0:
                with scope("ph_1_wait_x"):
                    cp_x(c).wait()
            if c + 1 < xch:
                cp_x(c + 1).start()
            with scope("ph_2_pack_x"):
                pack_x(c)
        if lo == wob_it:
            start_late()
        do_relay = lo * aun >= rlag
        n_start = aun if lo < last_start else 0

        def body_p(it, carry, do_relay=do_relay, n_start=n_start):
            def dmas(k):
                if n_start:
                    start_w(it * aun + look + k)
                if do_relay:
                    wait_w(it * aun + k - rlag)
            if n_start or do_relay:
                _dma_block(aun, dmas)
            fill = []
            if do_relay:
                for k in range(aun):
                    fill += relay_pieces(it * aun + k - rlag)
            items = [f for k in range(aun) for f in aproj_items(it * aun + k)]
            _interleave(items, fill)
            return carry
        with scope("ph_3_aproj"):
            lax.fori_loop(lo, hi, body_p, 0)

    ri = lax.broadcasted_iota(jnp.int32, (L, L), 0)
    ci = lax.broadcasted_iota(jnp.int32, (L, L), 1)
    mask = (ri < M) | (ri >= ci)
    bscale = DHB ** -0.5 * LOG2E
    gate = gate_ref[...].astype(F32).reshape(1, D)
    nb_items = max(HB - wdef + lag3, HB + lag2 + (wdef + 3) // 4) if wdef else HB + lag3
    zero_blk = jnp.zeros((DHA, 128), BF)

    def b_stream(s, box):
        loc = dict(acc=None)
        qs, ks, vs, ps, os_ = {}, {}, {}, {}, {}
        xrows = _ds(s * SEG, SEG)

        def init():
            xs = _unpack(xu[_ds(s * (SEG // 2), SEG // 2), :]).astype(F32)
            loc["h"] = jnp.concatenate([box["mem"], xs], axis=0)
            gl = jnp.sum(xs * gate, axis=-1, keepdims=True)
            loc["gs"] = 1.0 / (1.0 + jnp.exp(-gl))
            g_s[xrows, :] = jnp.broadcast_to(loc["gs"], (SEG, 128))

        def wo_item(j, o):
            r = _nn(o, wob_v[j * DHB:(j + 1) * DHB, :])
            loc["acc"] = r if loc["acc"] is None else loc["acc"] + r

        def item(i):
            if i == 0:
                init()
            if i < HB:
                qkv = _nn(loc["h"], _unpack(w3[i]))
                qs[i] = qkv[:, 0:DHB]
                ks[i] = qkv[:, DHB:2 * DHB].astype(BF)
                vs[i] = qkv[:, 2 * DHB:3 * DHB].astype(BF)
            j = i - lag1
            if 0 <= j < HB:
                sc = _nt(qs.pop(j), ks.pop(j))
                t = jnp.where(mask, sc * bscale, -1e9 * LOG2E)
                m = jnp.max(t, axis=-1, keepdims=True)
                p = jnp.exp2(t - m)
                l = jnp.sum(p, axis=-1, keepdims=True)
                ps[j] = p * (1.0 / l)
            j = i - lag2
            if 0 <= j < HB:
                o = _nn(ps.pop(j), vs.pop(j))
                if j >= HB - wdef:
                    o_buf[j - (HB - wdef)] = o
                else:
                    os_[j] = o
            j = i - lag3
            if 0 <= j < HB - wdef:
                wo_item(j, os_.pop(j))
            if wdef and i >= HB - 1 + lag2:
                k0 = i - (HB - 1 + lag2)
                n_left = nb_items - (HB - 1 + lag2)
                for jj in range(k0 * wdef // n_left, (k0 + 1) * wdef // n_left):
                    wo_item(HB - wdef + jj, o_buf[jj])
            if i == nb_items - 1:
                out = loc["acc"]
                b_s[xrows, :] = out[M:, :] * (1.0 - loc["gs"])
                box["mem"] = out[:M, :]
        return [functools.partial(item, i) for i in range(nb_items)]

    if cfg["order"] == "hc":
        work = [(b, ch) for b in (0, 4) for ch in range(NQ)]
    else:
        work = [(b, ch) for ch in range(NQ) for b in (0, 4)]
    na_items = len(work) + alag

    def masked_qt(g, qcols, hh):
        qh = _unpack(qt_u[_ds(g * 64 + hh * 8, 8), qcols])
        return jnp.concatenate([zero_blk] * hh + [qh] + [zero_blk] * (7 - hh), axis=0)

    def a_stream(sa, box):
        g, qt = sa % 4, sa // 4
        qcols = _ds(qt * 128, 128)
        pts, accs, ls, qms = {}, {}, {}, {}

        def item(i):
            if i == 0:
                for b in (0, 4):
                    qms[b] = jnp.concatenate([masked_qt(g, qcols, b + u) for u in range(4)], axis=1)
            if i < len(work):
                b, ch = work[i]
                sT = _nn(_unpack(k_u[g, ch * 64:(ch + 1) * 64, :]), qms[b])
                p = jnp.exp2(sT)
                lp = p[0:8]
                for r in range(1, 16):
                    lp = lp + p[8 * r:8 * r + 8]
                ls[b] = lp if ch == 0 else ls[b] + lp
                pts[i] = p.astype(BF)
            j = i - alag
            if j >= 0:
                b, ch = work[j]
                pj = pts.pop(j)
                for u in range(4):
                    urow = _ds(g * 64 + (b + u) * 8, 8)
                    r = _nn(_unpack(vt_u[urow, ch * 128:(ch + 1) * 128]), pj[:, u * 128:(u + 1) * 128])
                    accs[b + u] = r if ch == 0 else accs[b + u] + r
                    if ch == NQ - 1:
                        o = accs.pop(b + u)
                        l = jnp.sum(ls[b][:, u * 128:(u + 1) * 128], axis=0, keepdims=True)
                        ot_s[_ds(g * 128 + (b + u) * DHA, DHA), qcols] = (o * (1.0 / l)).astype(BF)
                        ok = (l >= L_LO) & (l <= L_HI)
                        bad_o = jnp.where(jnp.abs(o) < O_HI, 0.0, 1.0)
                        box["bad"] = jnp.maximum(box["bad"], jnp.maximum(
                            jnp.where(ok, 0.0, 1.0), jnp.maximum(bad_o[0:8], bad_o[8:16])))
        return [functools.partial(item, i) for i in range(na_items)]

    def run_ab(bs, as_, nun):
        nf, ns = len(bs), len(as_)
        lead, ramp = cfg["lead"], cfg["ramp"]
        si = 0
        for fi in range(nf):
            pos = fi / nf * nun
            edge = min(pos, nun - pos, ramp) / ramp
            target = (pos + lead * edge) / nun * ns
            while si < ns and si <= target:
                as_[si]()
                si += 1
            bs[fi]()
        while si < ns:
            as_[si]()
            si += 1

    def body(sb_list, sa_list, carry, fill=()):
        box = dict(mem=carry[0], bad=carry[1])
        bs = [it for sb in sb_list for it in b_stream(sb, box)]
        as_ = [it for sa in sa_list for it in a_stream(sa, box)]
        if bs and as_:
            run_ab(bs, as_, len(sb_list))
        else:
            _interleave(bs or as_, list(fill))
        return box["mem"], box["bad"]

    carry = (mem_ref[...].astype(F32), jnp.zeros((8, 128), F32))

    first_left = NQ - rlag
    with scope("ph_4w"):
        _dma_block(NW - first_left, lambda k: wait_w(first_left + k))
    if cfg["wob_at"] < 0:
        start_late()
    with scope("ph_4_pre"):
        fill = [f for j in range(first_left, NW) for f in relay_pieces(j)]
        for t in range(npre):
            carry = body([], [t], carry, fill[t * len(fill) // npre:(t + 1) * len(fill) // npre])
    with scope("ph_5_wait_wob"):
        cp_wob.wait()

    n_main = (NSEG - npre) // un

    def step_u(t, c):
        return body([t * un + u for u in range(un)], [t * un + u + npre for u in range(un)], c)

    with scope("ph_6_main"):
        carry = lax.fori_loop(0, n_main, step_u, carry)
        rest = list(range(n_main * un, NSEG - npre))
        if rest:
            carry = body(rest, [r + npre for r in rest], carry)

    @pl.when(jnp.max(carry[1]) > 0.0)
    def _():
        row_head = lax.broadcasted_iota(jnp.int32, (128, 128), 0) // DHA
        ck = 256

        def safe_block(i, c):
            hh, qt = i // NQ, i % NQ
            g = hh // 8
            qcols = _ds(qt * 128, 128)
            qv = _unpack(qt_u[_ds(g * 64, 64), qcols])
            qm = jnp.where(row_head == hh % 8, qv, jnp.zeros_like(qv))

            def scores(ch):
                return _nn(_unpack(k_u[g, _ds(ch * (ck // 2), ck // 2), :]), qm)

            def pass1(ch, m):
                return jnp.maximum(m, jnp.max(scores(ch), axis=0, keepdims=True))
            m = lax.fori_loop(0, S // ck, pass1, jnp.full((1, 128), -jnp.inf, F32))

            def pass2(ch, acc):
                o, l = acc
                p = jnp.exp2(scores(ch) - m)
                vt = _unpack(vt_u[_ds(hh * 8, 8), _ds(ch * ck, ck)])
                return o + _nn(vt, p.astype(BF)), l + jnp.sum(p, axis=0, keepdims=True)
            o, l = lax.fori_loop(0, S // ck, pass2, (jnp.zeros((DHA, 128), F32), jnp.zeros((1, 128), F32)))
            ot_s[_ds(hh * DHA, DHA), qcols] = (o * (1.0 / l)).astype(BF)
            return c
        lax.fori_loop(0, HA * NQ, safe_block, 0)

    cp_woa.wait()

    def final_tile(t):
        rows = _ds(t * 128, 128)
        a = _nn(ot_s[:, rows].T, woa_v[...])
        gq = g_s[rows, :]
        gq4 = jnp.concatenate([gq] * (D // 128), axis=1)
        out_v[rows, :] = (gq4 * a + b_s[rows, :]).astype(BF)

    ready = (NSEG - npre) * SEG // 128
    split = [0, cfg["fsplit"], ready] if npre == 2 else [k * ready // npre for k in range(npre + 1)]
    with scope("ph_7_post"):
        for k in range(npre):
            tiles = range(split[k], split[k + 1])
            carry = body([NSEG - npre + k], [], carry, [functools.partial(final_tile, t) for t in tiles])
            _dma_block(len(tiles), lambda j, k=k: cp_out(split[k] + j).start())
        for t in range(ready, NQ):
            final_tile(t)
        _dma_block(NQ - ready, lambda j: cp_out(ready + j).start())

    def drain(t, c):
        cp_out(t).wait()
        return c
    with scope("ph_8_drain"):
        lax.fori_loop(0, NQ, drain, 0)


@functools.partial(jax.jit, static_argnames=("cfg",))
def _impl(A_x, A_wqkv, A_wo, B_mem0, B_Wq, B_Wk, B_Wv, B_Wo, gate_w, cfg=None):
    cfg = dict(CFG if cfg is None else dict(cfg))
    any_spec = pl.BlockSpec(memory_space=pl.ANY)
    vmem_spec = pl.BlockSpec(memory_space=pltpu.VMEM)
    out = pl.pallas_call(
        functools.partial(_kernel, cfg=cfg),
        out_shape=jax.ShapeDtypeStruct((S, D), BF),
        in_specs=[any_spec] * 7 + [vmem_spec, vmem_spec],
        out_specs=any_spec,
        scratch_shapes=[
            pltpu.VMEM((S, D), BF),
            pltpu.VMEM((D, 3 * D), BF),
            pltpu.VMEM((D, D), BF),
            pltpu.VMEM((3, D * HB, DHB), BF),
            pltpu.VMEM((HB * DHB, D), BF),
            pltpu.VMEM((S // 2, D), U32),
            pltpu.VMEM((2, D // 2, D), U32),
            pltpu.VMEM((D // 2, D), U32),
            pltpu.VMEM((HB, D // 2, 3 * DHB), U32),
            pltpu.VMEM((D // 2, S), U32),
            pltpu.VMEM((4, S // 2, 128), U32),
            pltpu.VMEM((D // 2, S), U32),
            pltpu.VMEM((D, S), BF),
            pltpu.VMEM((S, D), F32),
            pltpu.VMEM((S, 128), F32),
            pltpu.VMEM((S, D), BF),
            pltpu.VMEM((max(cfg["wdef"], 1), L, DHB), F32),
            pltpu.SemaphoreType.DMA((3,)),
            pltpu.SemaphoreType.DMA((4,)),
            pltpu.SemaphoreType.DMA((3 * NW,)),
            pltpu.SemaphoreType.DMA((NQ,)),
        ],
        compiler_params=pltpu.CompilerParams(vmem_limit_bytes=100 * 2 ** 20),
        name="gated_mix_kernel",
    )(A_x.reshape(S, D), A_wqkv, A_wo,
      B_Wq.reshape(D * HB, DHB), B_Wk.reshape(D * HB, DHB), B_Wv.reshape(D * HB, DHB),
      B_Wo.reshape(HB * DHB, D), B_mem0.reshape(M, D), gate_w)
    return out.reshape(1, S, D)


def pallas_gated_mix__mha_block__memory_aug_recurrent_mem_tr__prompt_kernel(
    A_x, A_wqkv, A_wo, B_x, B_mem0, B_Wq, B_Wk, B_Wv, B_Wo, B_seg_len, gate_w,
):
    del B_x
    if isinstance(B_seg_len, int):
        assert B_seg_len == SEG, "the kernel is specialised to seg_len == 32"
    return _impl(A_x, A_wqkv, A_wo, B_mem0, B_Wq, B_Wk, B_Wv, B_Wo, gate_w)
```

```python
import contextlib
import functools

import jax
import jax.numpy as jnp
import numpy as np
from jax import lax
from jax.experimental import pallas as pl
from jax.experimental.pallas import tpu as pltpu

BF = jnp.bfloat16
F32 = jnp.float32
U32 = jnp.uint32

S = 2048
D = 512
HA, DHA = 32, 16
HB, DHB = 32, 128
M = 8
SEG = 32
L = M + SEG
NSEG = S // SEG
NQ = S // 128
NW = 16
LOG2E = 1.4426950408889634
LO16, HI16 = np.uint32(0x0000FFFF), np.uint32(0xFFFF0000)

L_LO, L_HI, O_HI = 2.0 ** -30, 2.0 ** 60, 2.0 ** 120

CFG = dict(lag1=4, lag2=8, lag3=16, wdef=8, alag=2, order="hc", unroll=2, npre=2,
           aun=2, look=4, rlag=4, fsplit=14, pw=1, po=1, px=0, wos=1, pslice=0, peel=1, lead=0.0, ramp=0.5, scopes=0, pieces="par")


def _nt(a, b):
    return lax.dot_general(a, b, (((1,), (1,)), ((), ())), preferred_element_type=F32)


def _nn(a, b):
    return lax.dot_general(a, b, (((1,), (0,)), ((), ())), preferred_element_type=F32)


def _pack(v):
    return pltpu.bitcast(v, U32)


def _unpack(v):
    return pltpu.bitcast(v, BF)


def _ds(start, size):
    if isinstance(start, int):
        return pl.ds(start, size)
    return pl.ds(pl.multiple_of(start, size), size)


def _dma_block(n, fn):
    if isinstance(n, int) and n <= 0:
        return

    def body(k, c):
        fn(k)
        return c
    lax.fori_loop(0, n, body, 0)


def _interleave(first, second):
    nf, ns = len(first), len(second)
    si = 0
    for fi in range(nf):
        while si < ns and si * nf <= fi * ns:
            second[si]()
            si += 1
        first[fi]()
    while si < ns:
        second[si]()
        si += 1


def _kernel(x_hbm, wqkv_hbm, woa_hbm, wq_hbm, wk_hbm, wv_hbm, wob_hbm, mem_ref, gate_ref,
            out_hbm,
            x_v, wqkv_v, woa_v, wraw, wob_v, xu, wtu, wku, w3, qt_u, k_u, vt_u, ot_s, b_s, g_s,
            out_v, o_buf, in_sem, x_sem, w_sem, out_sem, wo_sem, *, cfg):
    lag1, lag2, lag3, wdef, alag = cfg["lag1"], cfg["lag2"], cfg["lag3"], cfg["wdef"], cfg["alag"]
    un, npre, aun, look, rlag = cfg["unroll"], cfg["npre"], cfg["aun"], cfg["look"], cfg["rlag"]
    scope = jax.named_scope if cfg["scopes"] else (lambda n: contextlib.nullcontext())
    xch = 4
    xr = S // xch

    w_src = (wq_hbm, wk_hbm, wv_hbm)
    wr = (D // NW) * HB

    def cp_x(c):
        return pltpu.make_async_copy(x_hbm.at[pl.ds(c * xr, xr), :], x_v.at[pl.ds(c * xr, xr), :], x_sem.at[c])

    def cp_w(j, i):
        rows = _ds(j * wr, wr)
        return pltpu.make_async_copy(w_src[i].at[rows, :], wraw.at[i, rows, :], w_sem.at[j * 3 + i])

    def start_w(j):
        for i in range(3):
            cp_w(j, i).start(priority=cfg["pw"])

    def wait_w(j):
        for i in range(3):
            cp_w(j, i).wait()

    cp_wqkv = pltpu.make_async_copy(wqkv_hbm, wqkv_v, in_sem.at[0])
    wos = cfg["wos"]
    wor = HB * DHB // wos

    def cp_wob(k):
        rows = _ds(k * wor, wor)
        return pltpu.make_async_copy(wob_hbm.at[rows, :], wob_v.at[rows, :], wo_sem.at[k])

    cp_woa = pltpu.make_async_copy(woa_hbm, woa_v, in_sem.at[2])

    def cp_out(t):
        rows = _ds(t * 128, 128)
        return pltpu.make_async_copy(out_v.at[rows, :], out_hbm.at[rows, :], out_sem.at[t])

    def start_late():
        _dma_block(wos, lambda k: cp_wob(k).start(priority=cfg["po"]))

    cp_wqkv.start()
    cp_x(0).start()
    with scope("ph_0_wait"):
        cp_wqkv.wait()
        cp_x(0).wait()
    for j in range(look):
        start_w(j)

    sub_id = lax.broadcasted_iota(jnp.int32, (8, 128), 0)

    def transpose8(vs):
        for dist in (4, 2, 1):
            keep = (sub_id & dist) == 0
            new = list(vs)
            for a in range(8):
                if a & dist == 0:
                    x, y = vs[a], vs[a + dist]
                    new[a] = jnp.where(keep, x, pltpu.roll(y, dist, 0))
                    new[a + dist] = jnp.where(keep, pltpu.roll(x, 8 - dist, 0), y)
            vs = new
        return vs

    def relay_piece(j, i, u, half, par):
        blk = j * 2 + u
        r0 = (blk * 512 if isinstance(blk, int) else pl.multiple_of(blk * 512, 512)) + 16 * half
        lst = []
        for r in range(8):
            w0 = _pack(wraw[i, pl.ds(r0 + (2 * r) * HB, 16), :])
            w1 = _pack(wraw[i, pl.ds(r0 + (2 * r + 1) * HB, 16), :])
            lst.append((w0 & LO16) | (w1 << 16) if par == 0 else (w0 >> 16) | (w1 & HI16))
        lst = transpose8(lst)
        for p in range(8):
            w3[16 * half + 2 * p + par, _ds(blk * 8, 8), i * DHB:(i + 1) * DHB] = lst[p]

    def relay_pieces(j):
        return [functools.partial(relay_piece, j, i, u, half, par)
                for i in range(3) for u in range(2) for half in range(2) for par in range(2)]

    qscale = DHA ** -0.5 * LOG2E
    wku[...] = _pack(wqkv_v[:, D:2 * D])

    def transpose_w(m, g, c):
        src = wqkv_v[c * 128:(c + 1) * 128, 2 * m * D + g * 128:2 * m * D + (g + 1) * 128]
        wtu[m, g * 64:(g + 1) * 64, c * 128:(c + 1) * 128] = _pack(src.T)

    tr_items = [functools.partial(transpose_w, m, g, c) for m in range(2) for g in range(4) for c in range(4)]
    if not cfg["peel"]:
        for f in tr_items:
            f()

    def pack_x(c):
        def body(t, carry):
            xu[_ds(c * (xr // 2) + t * 64, 64), :] = _pack(x_v[_ds(c * xr + t * 128, 128), :])
            return carry
        lax.fori_loop(0, xr // 128, body, 0)

    def aproj_items(t):
        cols = _ds(t * 128, 128)
        st = {}

        def xb():
            if "x" not in st:
                st["x"] = _unpack(xu[_ds(t * 64, 64), :])
            return st["x"]

        def qt(g):
            r = _nt(_unpack(wtu[0, g * 64:(g + 1) * 64, :]), xb()) * qscale
            qt_u[g * 64:(g + 1) * 64, cols] = _pack(r.astype(BF))

        def kk(g):
            r = _nn(xb(), _unpack(wku[:, g * 128:(g + 1) * 128]))
            k_u[g, _ds(t * 64, 64), :] = _pack(r.astype(BF))

        def vt(g):
            r = _nt(_unpack(wtu[1, g * 64:(g + 1) * 64, :]), xb())
            vt_u[g * 64:(g + 1) * 64, cols] = _pack(r.astype(BF))
        return ([functools.partial(kk, g) for g in range(4)],
                [functools.partial(f, g) for f in (qt, vt) for g in range(4)])

    nit = NQ // aun
    ipx = nit // xch
    assert rlag % aun == 0 and ipx >= 1

    def x_events(c):
        if c > 0:
            cp_x(c).wait()
        if c + 1 < xch:
            cp_x(c + 1).start(priority=cfg["px"])
        pack_x(c)

    def w_events(it, do_relay):
        def dmas(k):
            j = it * aun + look + k
            if isinstance(j, int):
                if j < NW:
                    start_w(j)
            else:
                pl.when(j < NW)(lambda: start_w(j))
            if do_relay:
                wait_w(it * aun + k - rlag)
        _dma_block(aun, dmas)

    def aproj_iter(it, do_relay, first=False):
        fill = []
        if do_relay:
            for k in range(aun):
                fill += relay_pieces(it * aun + k - rlag)
        parts = [aproj_items(it * aun + k) for k in range(aun)]
        if first:
            _interleave([f for p in parts for f in p[0]], tr_items)
            _interleave([f for p in parts for f in p[1]], fill)
        else:
            _interleave([f for p in parts for f in p[0] + p[1]], fill)

    n_head = rlag // aun
    with scope("ph_3_aproj"):
        for it in range(n_head):
            if it % ipx == 0:
                x_events(it // ipx)
            w_events(it, False)
            aproj_iter(it, False, first=bool(cfg["peel"]) and it == 0)

        def body_p(it, carry):
            for c in range(1, xch):
                if c * ipx >= n_head:
                    pl.when(it == c * ipx)(functools.partial(x_events, c))
            w_events(it, True)
            aproj_iter(it, True)
            return carry
        lax.fori_loop(n_head, nit, body_p, 0)

    ri = lax.broadcasted_iota(jnp.int32, (L, L), 0)
    ci = lax.broadcasted_iota(jnp.int32, (L, L), 1)
    mask = (ri < M) | (ri >= ci)
    bscale = DHB ** -0.5 * LOG2E
    gate = gate_ref[...].astype(F32).reshape(1, D)
    nb_items = max(HB - wdef + lag3, HB + lag2 + (wdef + 3) // 4) if wdef else HB + lag3
    zero_blk = jnp.zeros((DHA, 128), BF)

    def b_stream(s, box):
        loc = dict(acc=None)
        qs, ks, vs, ps, os_ = {}, {}, {}, {}, {}
        xrows = _ds(s * SEG, SEG)

        def init():
            xs = _unpack(xu[_ds(s * (SEG // 2), SEG // 2), :]).astype(F32)
            loc["h"] = jnp.concatenate([box["mem"], xs], axis=0)
            gl = jnp.sum(xs * gate, axis=-1, keepdims=True)
            loc["gs"] = 1.0 / (1.0 + jnp.exp(-gl))
            g_s[xrows, :] = jnp.broadcast_to(loc["gs"], (SEG, 128))

        def wo_item(j, o):
            r = _nn(o, wob_v[j * DHB:(j + 1) * DHB, :])
            loc["acc"] = r if loc["acc"] is None else loc["acc"] + r

        def item(i):
            if i == 0:
                init()
            if i < HB:
                qkv = _nn(loc["h"], _unpack(w3[i]))
                qs[i] = qkv[:, 0:DHB]
                ks[i] = qkv[:, DHB:2 * DHB].astype(BF)
                vs[i] = qkv[:, 2 * DHB:3 * DHB].astype(BF)
            j = i - lag1
            if 0 <= j < HB:
                sc = _nt(qs.pop(j), ks.pop(j))
                t = jnp.where(mask, sc * bscale, -1e9 * LOG2E)
                m = jnp.max(t, axis=-1, keepdims=True)
                p = jnp.exp2(t - m)
                l = jnp.sum(p, axis=-1, keepdims=True)
                ps[j] = p * (1.0 / l)
            j = i - lag2
            if 0 <= j < HB:
                o = _nn(ps.pop(j), vs.pop(j))
                if j >= HB - wdef:
                    o_buf[j - (HB - wdef)] = o
                else:
                    os_[j] = o
            j = i - lag3
            if 0 <= j < HB - wdef:
                wo_item(j, os_.pop(j))
            if wdef and i >= HB - 1 + lag2:
                k0 = i - (HB - 1 + lag2)
                n_left = nb_items - (HB - 1 + lag2)
                for jj in range(k0 * wdef // n_left, (k0 + 1) * wdef // n_left):
                    wo_item(HB - wdef + jj, o_buf[jj])
            if i == nb_items - 1:
                out = loc["acc"]
                b_s[xrows, :] = out[M:, :] * (1.0 - loc["gs"])
                box["mem"] = out[:M, :]
        return [functools.partial(item, i) for i in range(nb_items)]

    if cfg["order"] == "hc":
        work = [(b, ch) for b in (0, 4) for ch in range(NQ)]
    else:
        work = [(b, ch) for ch in range(NQ) for b in (0, 4)]
    na_items = len(work) + alag

    def masked_qt(g, qcols, hh):
        qh = _unpack(qt_u[_ds(g * 64 + hh * 8, 8), qcols])
        return jnp.concatenate([zero_blk] * hh + [qh] + [zero_blk] * (7 - hh), axis=0)

    def a_stream(sa, box):
        g, qt = sa % 4, sa // 4
        qcols = _ds(qt * 128, 128)
        pts, accs, ls, qms = {}, {}, {}, {}

        def item(i):
            if i == 0:
                for b in (0, 4):
                    qms[b] = jnp.concatenate([masked_qt(g, qcols, b + u) for u in range(4)], axis=1)
            if i < len(work):
                b, ch = work[i]
                sT = _nn(_unpack(k_u[g, ch * 64:(ch + 1) * 64, :]), qms[b])
                p = jnp.exp2(sT)
                lp = p[0:8]
                for r in range(1, 16):
                    lp = lp + p[8 * r:8 * r + 8]
                ls[b] = lp if ch == 0 else ls[b] + lp
                pts[i] = [p[:, u * 128:(u + 1) * 128].astype(BF) for u in range(4)] if cfg["pslice"] else p.astype(BF)
            j = i - alag
            if j >= 0:
                b, ch = work[j]
                pj = pts.pop(j)
                for u in range(4):
                    urow = _ds(g * 64 + (b + u) * 8, 8)
                    r = _nn(_unpack(vt_u[urow, ch * 128:(ch + 1) * 128]), pj[u] if cfg["pslice"] else pj[:, u * 128:(u + 1) * 128])
                    accs[b + u] = r if ch == 0 else accs[b + u] + r
                    if ch == NQ - 1:
                        o = accs.pop(b + u)
                        l = jnp.sum(ls[b][:, u * 128:(u + 1) * 128], axis=0, keepdims=True)
                        ot_s[_ds(g * 128 + (b + u) * DHA, DHA), qcols] = (o * (1.0 / l)).astype(BF)
                        ok = (l >= L_LO) & (l <= L_HI)
                        bad_o = jnp.where(jnp.abs(o) < O_HI, 0.0, 1.0)
                        box["bad"] = jnp.maximum(box["bad"], jnp.maximum(
                            jnp.where(ok, 0.0, 1.0), jnp.maximum(bad_o[0:8], bad_o[8:16])))
        return [functools.partial(item, i) for i in range(na_items)]

    def run_ab(bs, as_, nun):
        nf, ns = len(bs), len(as_)
        lead, ramp = cfg["lead"], cfg["ramp"]
        si = 0
        for fi in range(nf):
            pos = fi / nf * nun
            edge = min(pos, nun - pos, ramp) / ramp
            target = (pos + lead * edge) / nun * ns
            while si < ns and si <= target:
                as_[si]()
                si += 1
            bs[fi]()
        while si < ns:
            as_[si]()
            si += 1

    def body(sb_list, sa_list, carry, fill=()):
        box = dict(mem=carry[0], bad=carry[1])
        bs = [it for sb in sb_list for it in b_stream(sb, box)]
        as_ = [it for sa in sa_list for it in a_stream(sa, box)]
        if bs and as_:
            run_ab(bs, as_, len(sb_list))
        else:
            _interleave(bs or as_, list(fill))
        return box["mem"], box["bad"]

    carry = (mem_ref[...].astype(F32), jnp.zeros((8, 128), F32))

    first_left = NQ - rlag
    start_late()
    n_left = NW - first_left
    with scope("ph_4_pre"):
        for t in range(npre):
            lo_, hi_ = first_left + t * n_left // npre, first_left + (t + 1) * n_left // npre
            with scope("ph_4w%d" % t):
                _dma_block(hi_ - lo_, lambda k, lo_=lo_: wait_w(lo_ + k))
            carry = body([], [t], carry, [f for j in range(lo_, hi_) for f in relay_pieces(j)])
    with scope("ph_5_wait_wob"):
        _dma_block(wos, lambda k: cp_wob(k).wait())
    cp_woa.start(priority=cfg["po"])

    n_main = (NSEG - npre) // un

    def step_u(t, c):
        return body([t * un + u for u in range(un)], [t * un + u + npre for u in range(un)], c)

    with scope("ph_6_main"):
        carry = lax.fori_loop(0, n_main, step_u, carry)
        rest = list(range(n_main * un, NSEG - npre))
        if rest:
            carry = body(rest, [r + npre for r in rest], carry)

    @pl.when(jnp.max(carry[1]) > 0.0)
    def _():
        row_head = lax.broadcasted_iota(jnp.int32, (128, 128), 0) // DHA
        ck = 256

        def safe_block(i, c):
            hh, qt = i // NQ, i % NQ
            g = hh // 8
            qcols = _ds(qt * 128, 128)
            qv = _unpack(qt_u[_ds(g * 64, 64), qcols])
            qm = jnp.where(row_head == hh % 8, qv, jnp.zeros_like(qv))

            def scores(ch):
                return _nn(_unpack(k_u[g, _ds(ch * (ck // 2), ck // 2), :]), qm)

            def pass1(ch, m):
                return jnp.maximum(m, jnp.max(scores(ch), axis=0, keepdims=True))
            m = lax.fori_loop(0, S // ck, pass1, jnp.full((1, 128), -jnp.inf, F32))

            def pass2(ch, acc):
                o, l = acc
                p = jnp.exp2(scores(ch) - m)
                vt = _unpack(vt_u[_ds(hh * 8, 8), _ds(ch * ck, ck)])
                return o + _nn(vt, p.astype(BF)), l + jnp.sum(p, axis=0, keepdims=True)
            o, l = lax.fori_loop(0, S // ck, pass2, (jnp.zeros((DHA, 128), F32), jnp.zeros((1, 128), F32)))
            ot_s[_ds(hh * DHA, DHA), qcols] = (o * (1.0 / l)).astype(BF)
            return c
        lax.fori_loop(0, HA * NQ, safe_block, 0)

    cp_woa.wait()

    def final_tile(t):
        rows = _ds(t * 128, 128)
        a = _nn(ot_s[:, rows].T, woa_v[...])
        gq = g_s[rows, :]
        gq4 = jnp.concatenate([gq] * (D // 128), axis=1)
        out_v[rows, :] = (gq4 * a + b_s[rows, :]).astype(BF)

    ready = (NSEG - npre) * SEG // 128
    split = [0, cfg["fsplit"], ready] if npre == 2 else [k * ready // npre for k in range(npre + 1)]
    with scope("ph_7_post"):
        for k in range(npre):
            tiles = range(split[k], split[k + 1])
            carry = body([NSEG - npre + k], [], carry, [functools.partial(final_tile, t) for t in tiles])
            _dma_block(len(tiles), lambda j, k=k: cp_out(split[k] + j).start())
        for t in range(ready, NQ):
            final_tile(t)
        _dma_block(NQ - ready, lambda j: cp_out(ready + j).start())

    def drain(t, c):
        cp_out(t).wait()
        return c
    with scope("ph_8_drain"):
        lax.fori_loop(0, NQ, drain, 0)


@functools.partial(jax.jit, static_argnames=("cfg",))
def _impl(A_x, A_wqkv, A_wo, B_mem0, B_Wq, B_Wk, B_Wv, B_Wo, gate_w, cfg=None):
    cfg = dict(CFG if cfg is None else dict(cfg))
    any_spec = pl.BlockSpec(memory_space=pl.ANY)
    vmem_spec = pl.BlockSpec(memory_space=pltpu.VMEM)
    out = pl.pallas_call(
        functools.partial(_kernel, cfg=cfg),
        out_shape=jax.ShapeDtypeStruct((S, D), BF),
        in_specs=[any_spec] * 7 + [vmem_spec, vmem_spec],
        out_specs=any_spec,
        scratch_shapes=[
            pltpu.VMEM((S, D), BF),
            pltpu.VMEM((D, 3 * D), BF),
            pltpu.VMEM((D, D), BF),
            pltpu.VMEM((3, D * HB, DHB), BF),
            pltpu.VMEM((HB * DHB, D), BF),
            pltpu.VMEM((S // 2, D), U32),
            pltpu.VMEM((2, D // 2, D), U32),
            pltpu.VMEM((D // 2, D), U32),
            pltpu.VMEM((HB, D // 2, 3 * DHB), U32),
            pltpu.VMEM((D // 2, S), U32),
            pltpu.VMEM((4, S // 2, 128), U32),
            pltpu.VMEM((D // 2, S), U32),
            pltpu.VMEM((D, S), BF),
            pltpu.VMEM((S, D), F32),
            pltpu.VMEM((S, 128), F32),
            pltpu.VMEM((S, D), BF),
            pltpu.VMEM((max(cfg["wdef"], 1), L, DHB), F32),
            pltpu.SemaphoreType.DMA((3,)),
            pltpu.SemaphoreType.DMA((4,)),
            pltpu.SemaphoreType.DMA((3 * NW,)),
            pltpu.SemaphoreType.DMA((NQ,)),
            pltpu.SemaphoreType.DMA((cfg["wos"],)),
        ],
        compiler_params=pltpu.CompilerParams(vmem_limit_bytes=100 * 2 ** 20),
        name="gated_mix_kernel",
    )(A_x.reshape(S, D), A_wqkv, A_wo,
      B_Wq.reshape(D * HB, DHB), B_Wk.reshape(D * HB, DHB), B_Wv.reshape(D * HB, DHB),
      B_Wo.reshape(HB * DHB, D), B_mem0.reshape(M, D), gate_w)
    return out.reshape(1, S, D)


def pallas_gated_mix__mha_block__memory_aug_recurrent_mem_tr__prompt_kernel(
    A_x, A_wqkv, A_wo, B_x, B_mem0, B_Wq, B_Wk, B_Wv, B_Wo, B_seg_len, gate_w,
):
    del B_x
    if isinstance(B_seg_len, int):
        assert B_seg_len == SEG, "the kernel is specialised to seg_len == 32"
    return _impl(A_x, A_wqkv, A_wo, B_mem0, B_Wq, B_Wk, B_Wv, B_Wo, gate_w)
```

```python
import functools

import jax
import jax.numpy as jnp
import numpy as np
from jax import lax
from jax.experimental import pallas as pl
from jax.experimental.pallas import tpu as pltpu

BF = jnp.bfloat16
F32 = jnp.float32
U32 = jnp.uint32

S = 2048
D = 512
HA, DHA = 32, 16
HB, DHB = 32, 128
M = 8
SEG = 32
L = M + SEG
NSEG = S // SEG
NQ = S // 128
NW = 16
LOG2E = 1.4426950408889634
LO16, HI16 = np.uint32(0x0000FFFF), np.uint32(0xFFFF0000)

L_LO, L_HI, O_HI = 2.0 ** -30, 2.0 ** 60, 2.0 ** 120

LAG_S, LAG_PV, LAG_WO = 4, 8, 16
WO_DEFER = 8
LAG_A = 2
UNROLL = 2
NPRE = 2
AUN = 2
LOOK = 4
RLAG = 4
FSPLIT = 14


def _nt(a, b):
    return lax.dot_general(a, b, (((1,), (1,)), ((), ())), preferred_element_type=F32)


def _nn(a, b):
    return lax.dot_general(a, b, (((1,), (0,)), ((), ())), preferred_element_type=F32)


def _pack(v):
    return pltpu.bitcast(v, U32)


def _unpack(v):
    return pltpu.bitcast(v, BF)


def _ds(start, size):
    if isinstance(start, int):
        return pl.ds(start, size)
    return pl.ds(pl.multiple_of(start, size), size)


def _dma_block(n, fn):
    if isinstance(n, int) and n <= 0:
        return

    def body(k, c):
        fn(k)
        return c
    lax.fori_loop(0, n, body, 0)


def _interleave(first, second):
    nf, ns = len(first), len(second)
    si = 0
    for fi in range(nf):
        while si < ns and si * nf <= fi * ns:
            second[si]()
            si += 1
        first[fi]()
    while si < ns:
        second[si]()
        si += 1


def _kernel(x_hbm, wqkv_hbm, woa_hbm, wq_hbm, wk_hbm, wv_hbm, wob_hbm, mem_ref, gate_ref,
            out_hbm,
            x_v, wqkv_v, woa_v, wraw, wob_v, xu, wtu, wku, w3, qt_u, k_u, vt_u, ot_s, b_s, g_s,
            out_v, o_buf, in_sem, x_sem, w_sem, out_sem):
    lag1, lag2, lag3, wdef, alag = LAG_S, LAG_PV, LAG_WO, WO_DEFER, LAG_A
    un, npre, aun, look, rlag = UNROLL, NPRE, AUN, LOOK, RLAG
    xch = 4
    xr = S // xch

    w_src = (wq_hbm, wk_hbm, wv_hbm)
    wr = (D // NW) * HB

    def cp_x(c):
        return pltpu.make_async_copy(x_hbm.at[pl.ds(c * xr, xr), :], x_v.at[pl.ds(c * xr, xr), :], x_sem.at[c])

    def cp_w(j, i):
        rows = _ds(j * wr, wr)
        return pltpu.make_async_copy(w_src[i].at[rows, :], wraw.at[i, rows, :], w_sem.at[j * 3 + i])

    def start_w(j):
        for i in range(3):
            cp_w(j, i).start(priority=1)

    def wait_w(j):
        for i in range(3):
            cp_w(j, i).wait()

    cp_wqkv = pltpu.make_async_copy(wqkv_hbm, wqkv_v, in_sem.at[0])
    cp_wob = pltpu.make_async_copy(wob_hbm, wob_v, in_sem.at[1])
    cp_woa = pltpu.make_async_copy(woa_hbm, woa_v, in_sem.at[2])

    def cp_out(t):
        rows = _ds(t * 128, 128)
        return pltpu.make_async_copy(out_v.at[rows, :], out_hbm.at[rows, :], out_sem.at[t])

    cp_wqkv.start()
    cp_x(0).start()
    cp_wqkv.wait()
    cp_x(0).wait()
    for j in range(look):
        start_w(j)

    sub_id = lax.broadcasted_iota(jnp.int32, (8, 128), 0)

    def transpose8(vs):
        for dist in (4, 2, 1):
            keep = (sub_id & dist) == 0
            new = list(vs)
            for a in range(8):
                if a & dist == 0:
                    x, y = vs[a], vs[a + dist]
                    new[a] = jnp.where(keep, x, pltpu.roll(y, dist, 0))
                    new[a + dist] = jnp.where(keep, pltpu.roll(x, 8 - dist, 0), y)
            vs = new
        return vs

    def relay_piece(j, i, u, half, par):
        blk = j * 2 + u
        r0 = (blk * 512 if isinstance(blk, int) else pl.multiple_of(blk * 512, 512)) + 16 * half
        lst = []
        for r in range(8):
            w0 = _pack(wraw[i, pl.ds(r0 + (2 * r) * HB, 16), :])
            w1 = _pack(wraw[i, pl.ds(r0 + (2 * r + 1) * HB, 16), :])
            lst.append((w0 & LO16) | (w1 << 16) if par == 0 else (w0 >> 16) | (w1 & HI16))
        lst = transpose8(lst)
        for p in range(8):
            w3[16 * half + 2 * p + par, _ds(blk * 8, 8), i * DHB:(i + 1) * DHB] = lst[p]

    def relay_pieces(j):
        return [functools.partial(relay_piece, j, i, u, half, par)
                for i in range(3) for u in range(2) for half in range(2) for par in range(2)]

    qscale = DHA ** -0.5 * LOG2E
    wku[...] = _pack(wqkv_v[:, D:2 * D])

    def transpose_w(m, g, c):
        src = wqkv_v[c * 128:(c + 1) * 128, 2 * m * D + g * 128:2 * m * D + (g + 1) * 128]
        wtu[m, g * 64:(g + 1) * 64, c * 128:(c + 1) * 128] = _pack(src.T)

    tr_items = [functools.partial(transpose_w, m, g, c) for m in range(2) for g in range(4) for c in range(4)]

    def pack_x(c):
        def body(t, carry):
            xu[_ds(c * (xr // 2) + t * 64, 64), :] = _pack(x_v[_ds(c * xr + t * 128, 128), :])
            return carry
        lax.fori_loop(0, xr // 128, body, 0)

    def aproj_items(t):
        cols = _ds(t * 128, 128)
        st = {}

        def xb():
            if "x" not in st:
                st["x"] = _unpack(xu[_ds(t * 64, 64), :])
            return st["x"]

        def qt(g):
            r = _nt(_unpack(wtu[0, g * 64:(g + 1) * 64, :]), xb()) * qscale
            qt_u[g * 64:(g + 1) * 64, cols] = _pack(r.astype(BF))

        def kk(g):
            r = _nn(xb(), _unpack(wku[:, g * 128:(g + 1) * 128]))
            k_u[g, _ds(t * 64, 64), :] = _pack(r.astype(BF))

        def vt(g):
            r = _nt(_unpack(wtu[1, g * 64:(g + 1) * 64, :]), xb())
            vt_u[g * 64:(g + 1) * 64, cols] = _pack(r.astype(BF))
        return ([functools.partial(kk, g) for g in range(4)],
                [functools.partial(f, g) for f in (qt, vt) for g in range(4)])

    nit = NQ // aun
    ipx = nit // xch
    assert rlag % aun == 0 and ipx >= 1

    def x_events(c):
        if c > 0:
            cp_x(c).wait()
        if c + 1 < xch:
            cp_x(c + 1).start()
        pack_x(c)

    def w_events(it, do_relay):
        def dmas(k):
            j = it * aun + look + k
            if isinstance(j, int):
                if j < NW:
                    start_w(j)
            else:
                pl.when(j < NW)(lambda: start_w(j))
            if do_relay:
                wait_w(it * aun + k - rlag)
        _dma_block(aun, dmas)

    def aproj_iter(it, do_relay, first=False):
        fill = []
        if do_relay:
            for k in range(aun):
                fill += relay_pieces(it * aun + k - rlag)
        parts = [aproj_items(it * aun + k) for k in range(aun)]
        if first:
            _interleave([f for p in parts for f in p[0]], tr_items)
            _interleave([f for p in parts for f in p[1]], fill)
        else:
            _interleave([f for p in parts for f in p[0] + p[1]], fill)

    n_head = rlag // aun
    for it in range(n_head):
        if it % ipx == 0:
            x_events(it // ipx)
        w_events(it, False)
        aproj_iter(it, False, first=it == 0)

    def body_p(it, carry):
        for c in range(1, xch):
            if c * ipx >= n_head:
                pl.when(it == c * ipx)(functools.partial(x_events, c))
        w_events(it, True)
        aproj_iter(it, True)
        return carry
    lax.fori_loop(n_head, nit, body_p, 0)

    ri = lax.broadcasted_iota(jnp.int32, (L, L), 0)
    ci = lax.broadcasted_iota(jnp.int32, (L, L), 1)
    mask = (ri < M) | (ri >= ci)
    bscale = DHB ** -0.5 * LOG2E
    gate = gate_ref[...].astype(F32).reshape(1, D)
    nb_items = max(HB - wdef + lag3, HB + lag2 + (wdef + 3) // 4) if wdef else HB + lag3
    zero_blk = jnp.zeros((DHA, 128), BF)

    def b_stream(s, box):
        loc = dict(acc=None)
        qs, ks, vs, ps, os_ = {}, {}, {}, {}, {}
        xrows = _ds(s * SEG, SEG)

        def init():
            xs = _unpack(xu[_ds(s * (SEG // 2), SEG // 2), :]).astype(F32)
            loc["h"] = jnp.concatenate([box["mem"], xs], axis=0)
            gl = jnp.sum(xs * gate, axis=-1, keepdims=True)
            loc["gs"] = 1.0 / (1.0 + jnp.exp(-gl))
            g_s[xrows, :] = jnp.broadcast_to(loc["gs"], (SEG, 128))

        def wo_item(j, o):
            r = _nn(o, wob_v[j * DHB:(j + 1) * DHB, :])
            loc["acc"] = r if loc["acc"] is None else loc["acc"] + r

        def item(i):
            if i == 0:
                init()
            if i < HB:
                qkv = _nn(loc["h"], _unpack(w3[i]))
                qs[i] = qkv[:, 0:DHB]
                ks[i] = qkv[:, DHB:2 * DHB].astype(BF)
                vs[i] = qkv[:, 2 * DHB:3 * DHB].astype(BF)
            j = i - lag1
            if 0 <= j < HB:
                sc = _nt(qs.pop(j), ks.pop(j))
                t = jnp.where(mask, sc * bscale, -1e9 * LOG2E)
                m = jnp.max(t, axis=-1, keepdims=True)
                p = jnp.exp2(t - m)
                l = jnp.sum(p, axis=-1, keepdims=True)
                ps[j] = p * (1.0 / l)
            j = i - lag2
            if 0 <= j < HB:
                o = _nn(ps.pop(j), vs.pop(j))
                if j >= HB - wdef:
                    o_buf[j - (HB - wdef)] = o
                else:
                    os_[j] = o
            j = i - lag3
            if 0 <= j < HB - wdef:
                wo_item(j, os_.pop(j))
            if wdef and i >= HB - 1 + lag2:
                k0 = i - (HB - 1 + lag2)
                n_left = nb_items - (HB - 1 + lag2)
                for jj in range(k0 * wdef // n_left, (k0 + 1) * wdef // n_left):
                    wo_item(HB - wdef + jj, o_buf[jj])
            if i == nb_items - 1:
                out = loc["acc"]
                b_s[xrows, :] = out[M:, :] * (1.0 - loc["gs"])
                box["mem"] = out[:M, :]
        return [functools.partial(item, i) for i in range(nb_items)]

    work = [(b, ch) for b in (0, 4) for ch in range(NQ)]
    na_items = len(work) + alag

    def masked_qt(g, qcols, hh):
        qh = _unpack(qt_u[_ds(g * 64 + hh * 8, 8), qcols])
        return jnp.concatenate([zero_blk] * hh + [qh] + [zero_blk] * (7 - hh), axis=0)

    def a_stream(sa, box):
        g, qt = sa % 4, sa // 4
        qcols = _ds(qt * 128, 128)
        pts, accs, ls, qms = {}, {}, {}, {}

        def item(i):
            if i == 0:
                for b in (0, 4):
                    qms[b] = jnp.concatenate([masked_qt(g, qcols, b + u) for u in range(4)], axis=1)
            if i < len(work):
                b, ch = work[i]
                sT = _nn(_unpack(k_u[g, ch * 64:(ch + 1) * 64, :]), qms[b])
                p = jnp.exp2(sT)
                lp = p[0:8]
                for r in range(1, 16):
                    lp = lp + p[8 * r:8 * r + 8]
                ls[b] = lp if ch == 0 else ls[b] + lp
                pts[i] = p.astype(BF)
            j = i - alag
            if j >= 0:
                b, ch = work[j]
                pj = pts.pop(j)
                for u in range(4):
                    urow = _ds(g * 64 + (b + u) * 8, 8)
                    r = _nn(_unpack(vt_u[urow, ch * 128:(ch + 1) * 128]), pj[:, u * 128:(u + 1) * 128])
                    accs[b + u] = r if ch == 0 else accs[b + u] + r
                    if ch == NQ - 1:
                        o = accs.pop(b + u)
                        l = jnp.sum(ls[b][:, u * 128:(u + 1) * 128], axis=0, keepdims=True)
                        ot_s[_ds(g * 128 + (b + u) * DHA, DHA), qcols] = (o * (1.0 / l)).astype(BF)
                        ok = (l >= L_LO) & (l <= L_HI)
                        bad_o = jnp.where(jnp.abs(o) < O_HI, 0.0, 1.0)
                        box["bad"] = jnp.maximum(box["bad"], jnp.maximum(
                            jnp.where(ok, 0.0, 1.0), jnp.maximum(bad_o[0:8], bad_o[8:16])))
        return [functools.partial(item, i) for i in range(na_items)]

    def body(sb_list, sa_list, carry, fill=()):
        box = dict(mem=carry[0], bad=carry[1])
        bs = [it for sb in sb_list for it in b_stream(sb, box)]
        as_ = [it for sa in sa_list for it in a_stream(sa, box)]
        if bs and as_:
            _interleave(bs, as_)
        else:
            _interleave(bs or as_, list(fill))
        return box["mem"], box["bad"]

    carry = (mem_ref[...].astype(F32), jnp.zeros((8, 128), F32))

    first_left = NQ - rlag
    _dma_block(1, lambda _: cp_wob.start(priority=1))
    n_left = NW - first_left
    for t in range(npre):
        lo_, hi_ = first_left + t * n_left // npre, first_left + (t + 1) * n_left // npre
        _dma_block(hi_ - lo_, lambda k, lo_=lo_: wait_w(lo_ + k))
        carry = body([], [t], carry, [f for j in range(lo_, hi_) for f in relay_pieces(j)])
    _dma_block(1, lambda _: cp_wob.wait())
    cp_woa.start(priority=1)

    n_main = (NSEG - npre) // un

    def step_u(t, c):
        return body([t * un + u for u in range(un)], [t * un + u + npre for u in range(un)], c)

    carry = lax.fori_loop(0, n_main, step_u, carry)

    @pl.when(jnp.max(carry[1]) > 0.0)
    def _():
        row_head = lax.broadcasted_iota(jnp.int32, (128, 128), 0) // DHA
        ck = 256

        def safe_block(i, c):
            hh, qt = i // NQ, i % NQ
            g = hh // 8
            qcols = _ds(qt * 128, 128)
            qv = _unpack(qt_u[_ds(g * 64, 64), qcols])
            qm = jnp.where(row_head == hh % 8, qv, jnp.zeros_like(qv))

            def scores(ch):
                return _nn(_unpack(k_u[g, _ds(ch * (ck // 2), ck // 2), :]), qm)

            def pass1(ch, m):
                return jnp.maximum(m, jnp.max(scores(ch), axis=0, keepdims=True))
            m = lax.fori_loop(0, S // ck, pass1, jnp.full((1, 128), -jnp.inf, F32))

            def pass2(ch, acc):
                o, l = acc
                p = jnp.exp2(scores(ch) - m)
                vt = _unpack(vt_u[_ds(hh * 8, 8), _ds(ch * ck, ck)])
                return o + _nn(vt, p.astype(BF)), l + jnp.sum(p, axis=0, keepdims=True)
            o, l = lax.fori_loop(0, S // ck, pass2, (jnp.zeros((DHA, 128), F32), jnp.zeros((1, 128), F32)))
            ot_s[_ds(hh * DHA, DHA), qcols] = (o * (1.0 / l)).astype(BF)
            return c
        lax.fori_loop(0, HA * NQ, safe_block, 0)

    cp_woa.wait()

    def final_tile(t):
        rows = _ds(t * 128, 128)
        a = _nn(ot_s[:, rows].T, woa_v[...])
        gq = g_s[rows, :]
        gq4 = jnp.concatenate([gq] * (D // 128), axis=1)
        out_v[rows, :] = (gq4 * a + b_s[rows, :]).astype(BF)

    ready = (NSEG - npre) * SEG // 128
    split = [0, FSPLIT, ready]
    for k in range(npre):
        tiles = range(split[k], split[k + 1])
        carry = body([NSEG - npre + k], [], carry, [functools.partial(final_tile, t) for t in tiles])
        _dma_block(len(tiles), lambda j, k=k: cp_out(split[k] + j).start())
    for t in range(ready, NQ):
        final_tile(t)
    _dma_block(NQ - ready, lambda j: cp_out(ready + j).start())

    def drain(t, c):
        cp_out(t).wait()
        return c
    lax.fori_loop(0, NQ, drain, 0)


@jax.jit
def _impl(A_x, A_wqkv, A_wo, B_mem0, B_Wq, B_Wk, B_Wv, B_Wo, gate_w):
    any_spec = pl.BlockSpec(memory_space=pl.ANY)
    vmem_spec = pl.BlockSpec(memory_space=pltpu.VMEM)
    out = pl.pallas_call(
        _kernel,
        out_shape=jax.ShapeDtypeStruct((S, D), BF),
        in_specs=[any_spec] * 7 + [vmem_spec, vmem_spec],
        out_specs=any_spec,
        scratch_shapes=[
            pltpu.VMEM((S, D), BF),
            pltpu.VMEM((D, 3 * D), BF),
            pltpu.VMEM((D, D), BF),
            pltpu.VMEM((3, D * HB, DHB), BF),
            pltpu.VMEM((HB * DHB, D), BF),
            pltpu.VMEM((S // 2, D), U32),
            pltpu.VMEM((2, D // 2, D), U32),
            pltpu.VMEM((D // 2, D), U32),
            pltpu.VMEM((HB, D // 2, 3 * DHB), U32),
            pltpu.VMEM((D // 2, S), U32),
            pltpu.VMEM((4, S // 2, 128), U32),
            pltpu.VMEM((D // 2, S), U32),
            pltpu.VMEM((D, S), BF),
            pltpu.VMEM((S, D), F32),
            pltpu.VMEM((S, 128), F32),
            pltpu.VMEM((S, D), BF),
            pltpu.VMEM((WO_DEFER, L, DHB), F32),
            pltpu.SemaphoreType.DMA((3,)),
            pltpu.SemaphoreType.DMA((4,)),
            pltpu.SemaphoreType.DMA((3 * NW,)),
            pltpu.SemaphoreType.DMA((NQ,)),
        ],
        compiler_params=pltpu.CompilerParams(vmem_limit_bytes=100 * 2 ** 20),
        name="gated_mix_kernel",
    )(A_x.reshape(S, D), A_wqkv, A_wo,
      B_Wq.reshape(D * HB, DHB), B_Wk.reshape(D * HB, DHB), B_Wv.reshape(D * HB, DHB),
      B_Wo.reshape(HB * DHB, D), B_mem0.reshape(M, D), gate_w)
    return out.reshape(1, S, D)


def pallas_gated_mix__mha_block__memory_aug_recurrent_mem_tr__prompt_kernel(
    A_x, A_wqkv, A_wo, B_x, B_mem0, B_Wq, B_Wk, B_Wv, B_Wo, B_seg_len, gate_w,
):
    del B_x
    if isinstance(B_seg_len, int):
        assert B_seg_len == SEG, "the kernel is specialised to seg_len == 32"
    return _impl(A_x, A_wqkv, A_wo, B_mem0, B_Wq, B_Wk, B_Wv, B_Wo, gate_w)
```

```python
import functools

import jax
import jax.numpy as jnp
import numpy as np
from jax import lax
from jax.experimental import pallas as pl
from jax.experimental.pallas import tpu as pltpu

BF = jnp.bfloat16
F32 = jnp.float32
U32 = jnp.uint32

S = 2048
D = 512
HA, DHA = 32, 16
HB, DHB = 32, 128
M = 8
SEG = 32
L = M + SEG
NSEG = S // SEG
NQ = S // 128
NW = 16
LOG2E = 1.4426950408889634
LO16, HI16 = np.uint32(0x0000FFFF), np.uint32(0xFFFF0000)

L_LO, L_HI, O_HI = 2.0 ** -30, 2.0 ** 60, 2.0 ** 120

LAG_S, LAG_PV, LAG_WO = 3, 8, 18
WO_DEFER = 10
LAG_A = 2
UNROLL = 2
NPRE = 2
AUN = 2
LOOK = 4
RLAG = 4
FSPLIT = 14


def _nt(a, b):
    return lax.dot_general(a, b, (((1,), (1,)), ((), ())), preferred_element_type=F32)


def _nn(a, b):
    return lax.dot_general(a, b, (((1,), (0,)), ((), ())), preferred_element_type=F32)


def _pack(v):
    return pltpu.bitcast(v, U32)


def _unpack(v):
    return pltpu.bitcast(v, BF)


def _ds(start, size):
    if isinstance(start, int):
        return pl.ds(start, size)
    return pl.ds(pl.multiple_of(start, size), size)


def _dma_block(n, fn):
    if isinstance(n, int) and n <= 0:
        return

    def body(k, c):
        fn(k)
        return c
    lax.fori_loop(0, n, body, 0)


def _interleave(first, second):
    nf, ns = len(first), len(second)
    si = 0
    for fi in range(nf):
        while si < ns and si * nf <= fi * ns:
            second[si]()
            si += 1
        first[fi]()
    while si < ns:
        second[si]()
        si += 1


def _kernel(x_hbm, wqkv_hbm, woa_hbm, wq_hbm, wk_hbm, wv_hbm, wob_hbm, mem_ref, gate_ref,
            out_hbm,
            x_v, wqkv_v, woa_v, wraw, wob_v, xu, wtu, wku, w3, qt_u, k_u, vt_u, ot_s, b_s, g_s,
            out_v, o_buf, in_sem, x_sem, w_sem, out_sem):
    lag1, lag2, lag3, wdef, alag = LAG_S, LAG_PV, LAG_WO, WO_DEFER, LAG_A
    un, npre, aun, look, rlag = UNROLL, NPRE, AUN, LOOK, RLAG
    xch = 4
    xr = S // xch

    w_src = (wq_hbm, wk_hbm, wv_hbm)
    wr = (D // NW) * HB

    def cp_x(c):
        return pltpu.make_async_copy(x_hbm.at[pl.ds(c * xr, xr), :], x_v.at[pl.ds(c * xr, xr), :], x_sem.at[c])

    def cp_w(j, i):
        rows = _ds(j * wr, wr)
        return pltpu.make_async_copy(w_src[i].at[rows, :], wraw.at[i, rows, :], w_sem.at[j * 3 + i])

    def start_w(j):
        for i in range(3):
            cp_w(j, i).start(priority=1)

    def wait_w(j):
        for i in range(3):
            cp_w(j, i).wait()

    cp_wqkv = pltpu.make_async_copy(wqkv_hbm, wqkv_v, in_sem.at[0])
    cp_wob = pltpu.make_async_copy(wob_hbm, wob_v, in_sem.at[1])
    cp_woa = pltpu.make_async_copy(woa_hbm, woa_v, in_sem.at[2])

    def cp_out(t):
        rows = _ds(t * 128, 128)
        return pltpu.make_async_copy(out_v.at[rows, :], out_hbm.at[rows, :], out_sem.at[t])

    cp_wqkv.start()
    cp_x(0).start()
    cp_wqkv.wait()
    cp_x(0).wait()
    for j in range(look):
        start_w(j)

    sub_id = lax.broadcasted_iota(jnp.int32, (8, 128), 0)

    def transpose8(vs):
        for dist in (4, 2, 1):
            keep = (sub_id & dist) == 0
            new = list(vs)
            for a in range(8):
                if a & dist == 0:
                    x, y = vs[a], vs[a + dist]
                    new[a] = jnp.where(keep, x, pltpu.roll(y, dist, 0))
                    new[a + dist] = jnp.where(keep, pltpu.roll(x, 8 - dist, 0), y)
            vs = new
        return vs

    def relay_piece(j, i, u, half, par):
        blk = j * 2 + u
        r0 = (blk * 512 if isinstance(blk, int) else pl.multiple_of(blk * 512, 512)) + 16 * half
        lst = []
        for r in range(8):
            w0 = _pack(wraw[i, pl.ds(r0 + (2 * r) * HB, 16), :])
            w1 = _pack(wraw[i, pl.ds(r0 + (2 * r + 1) * HB, 16), :])
            lst.append((w0 & LO16) | (w1 << 16) if par == 0 else (w0 >> 16) | (w1 & HI16))
        lst = transpose8(lst)
        for p in range(8):
            w3[16 * half + 2 * p + par, _ds(blk * 8, 8), i * DHB:(i + 1) * DHB] = lst[p]

    def relay_pieces(j):
        return [functools.partial(relay_piece, j, i, u, half, par)
                for i in range(3) for u in range(2) for half in range(2) for par in range(2)]

    qscale = DHA ** -0.5 * LOG2E
    wku[...] = _pack(wqkv_v[:, D:2 * D])

    def transpose_w(m, g, c):
        src = wqkv_v[c * 128:(c + 1) * 128, 2 * m * D + g * 128:2 * m * D + (g + 1) * 128]
        wtu[m, g * 64:(g + 1) * 64, c * 128:(c + 1) * 128] = _pack(src.T)

    tr_items = [functools.partial(transpose_w, m, g, c) for m in range(2) for g in range(4) for c in range(4)]

    def pack_x(c):
        def body(t, carry):
            xu[_ds(c * (xr // 2) + t * 64, 64), :] = _pack(x_v[_ds(c * xr + t * 128, 128), :])
            return carry
        lax.fori_loop(0, xr // 128, body, 0)

    def aproj_items(t):
        cols = _ds(t * 128, 128)
        st = {}

        def xb():
            if "x" not in st:
                st["x"] = _unpack(xu[_ds(t * 64, 64), :])
            return st["x"]

        def qt(g):
            r = _nt(_unpack(wtu[0, g * 64:(g + 1) * 64, :]), xb()) * qscale
            qt_u[g * 64:(g + 1) * 64, cols] = _pack(r.astype(BF))

        def kk(g):
            r = _nn(xb(), _unpack(wku[:, g * 128:(g + 1) * 128]))
            k_u[g, _ds(t * 64, 64), :] = _pack(r.astype(BF))

        def vt(g):
            r = _nt(_unpack(wtu[1, g * 64:(g + 1) * 64, :]), xb())
            vt_u[g * 64:(g + 1) * 64, cols] = _pack(r.astype(BF))
        return ([functools.partial(kk, g) for g in range(4)],
                [functools.partial(f, g) for f in (qt, vt) for g in range(4)])

    nit = NQ // aun
    ipx = nit // xch
    assert rlag % aun == 0 and ipx >= 1

    def x_events(c):
        if c > 0:
            cp_x(c).wait()
        if c + 1 < xch:
            cp_x(c + 1).start()
        pack_x(c)

    def w_events(it, do_relay):
        def dmas(k):
            j = it * aun + look + k
            if isinstance(j, int):
                if j < NW:
                    start_w(j)
            else:
                pl.when(j < NW)(lambda: start_w(j))
            if do_relay:
                wait_w(it * aun + k - rlag)
        _dma_block(aun, dmas)

    def aproj_iter(it, do_relay, first=False):
        fill = []
        if do_relay:
            for k in range(aun):
                fill += relay_pieces(it * aun + k - rlag)
        parts = [aproj_items(it * aun + k) for k in range(aun)]
        if first:
            _interleave([f for p in parts for f in p[0]], tr_items)
            _interleave([f for p in parts for f in p[1]], fill)
        else:
            _interleave([f for p in parts for f in p[0] + p[1]], fill)

    n_head = rlag // aun
    for it in range(n_head):
        if it % ipx == 0:
            x_events(it // ipx)
        w_events(it, False)
        aproj_iter(it, False, first=it == 0)

    def body_p(it, carry):
        for c in range(1, xch):
            if c * ipx >= n_head:
                pl.when(it == c * ipx)(functools.partial(x_events, c))
        w_events(it, True)
        aproj_iter(it, True)
        return carry
    lax.fori_loop(n_head, nit, body_p, 0)

    ri = lax.broadcasted_iota(jnp.int32, (L, L), 0)
    ci = lax.broadcasted_iota(jnp.int32, (L, L), 1)
    mask = (ri < M) | (ri >= ci)
    bscale = DHB ** -0.5 * LOG2E
    gate = gate_ref[...].astype(F32).reshape(1, D)
    nb_items = max(HB - wdef + lag3, HB + lag2 + (wdef + 3) // 4)
    assert wdef // (nb_items - (HB - 1 + lag2)) < wdef
    zero_blk = jnp.zeros((DHA, 128), BF)

    def b_stream(s, box):
        loc = dict(acc=None)
        qs, ks, vs, ps, os_ = {}, {}, {}, {}, {}
        xrows = _ds(s * SEG, SEG)

        def init():
            xs = _unpack(xu[_ds(s * (SEG // 2), SEG // 2), :]).astype(F32)
            loc["h"] = jnp.concatenate([box["mem"], xs], axis=0)
            gl = jnp.sum(xs * gate, axis=-1, keepdims=True)
            loc["gs"] = 1.0 / (1.0 + jnp.exp(-gl))
            g_s[xrows, :] = jnp.broadcast_to(loc["gs"], (SEG, 128))

        def wo_item(j, o):
            r = _nn(o, wob_v[j * DHB:(j + 1) * DHB, :])
            loc["acc"] = r if loc["acc"] is None else loc["acc"] + r

        def item(i):
            if i == 0:
                init()
            j = i - lag3
            if 0 <= j < HB - wdef:
                wo_item(j, os_.pop(j))
            if i >= HB - 1 + lag2:
                k0 = i - (HB - 1 + lag2)
                n_left = nb_items - (HB - 1 + lag2)
                for jj in range(k0 * wdef // n_left, (k0 + 1) * wdef // n_left):
                    wo_item(HB - wdef + jj, o_buf[jj])
            j = i - lag1
            if 0 <= j < HB:
                sc = _nt(qs.pop(j), ks.pop(j))
                t = jnp.where(mask, sc * bscale, -1e9 * LOG2E)
                m = jnp.max(t, axis=-1, keepdims=True)
                p = jnp.exp2(t - m)
                l = jnp.sum(p, axis=-1, keepdims=True)
                ps[j] = p * (1.0 / l)
            j = i - lag2
            if 0 <= j < HB:
                o = _nn(ps.pop(j), vs.pop(j))
                if j >= HB - wdef:
                    o_buf[j - (HB - wdef)] = o
                else:
                    os_[j] = o
            if i < HB:
                qkv = _nn(loc["h"], _unpack(w3[i]))
                qs[i] = qkv[:, 0:DHB]
                ks[i] = qkv[:, DHB:2 * DHB].astype(BF)
                vs[i] = qkv[:, 2 * DHB:3 * DHB].astype(BF)
            if i == nb_items - 1:
                out = loc["acc"]
                b_s[xrows, :] = out[M:, :] * (1.0 - loc["gs"])
                box["mem"] = out[:M, :]
        return [functools.partial(item, i) for i in range(nb_items)]

    work = [(b, ch) for b in (0, 4) for ch in range(NQ)]
    na_items = len(work) + alag

    def masked_qt(g, qcols, hh):
        qh = _unpack(qt_u[_ds(g * 64 + hh * 8, 8), qcols])
        return jnp.concatenate([zero_blk] * hh + [qh] + [zero_blk] * (7 - hh), axis=0)

    def a_stream(sa, box):
        g, qt = sa % 4, sa // 4
        qcols = _ds(qt * 128, 128)
        pts, accs, ls, qms = {}, {}, {}, {}

        def item(i):
            if i == 0:
                for b in (0, 4):
                    qms[b] = jnp.concatenate([masked_qt(g, qcols, b + u) for u in range(4)], axis=1)
            if i < len(work):
                b, ch = work[i]
                sT = _nn(_unpack(k_u[g, ch * 64:(ch + 1) * 64, :]), qms[b])
                p = jnp.exp2(sT)
                lp = p[0:8]
                for r in range(1, 16):
                    lp = lp + p[8 * r:8 * r + 8]
                ls[b] = lp if ch == 0 else ls[b] + lp
                pts[i] = p.astype(BF)
            j = i - alag
            if j >= 0:
                b, ch = work[j]
                pj = pts.pop(j)
                for u in range(4):
                    urow = _ds(g * 64 + (b + u) * 8, 8)
                    r = _nn(_unpack(vt_u[urow, ch * 128:(ch + 1) * 128]), pj[:, u * 128:(u + 1) * 128])
                    accs[b + u] = r if ch == 0 else accs[b + u] + r
                    if ch == NQ - 1:
                        o = accs.pop(b + u)
                        l = jnp.sum(ls[b][:, u * 128:(u + 1) * 128], axis=0, keepdims=True)
                        ot_s[_ds(g * 128 + (b + u) * DHA, DHA), qcols] = (o * (1.0 / l)).astype(BF)
                        ok = (l >= L_LO) & (l <= L_HI)
                        bad_o = jnp.where(jnp.abs(o) < O_HI, 0.0, 1.0)
                        box["bad"] = jnp.maximum(box["bad"], jnp.maximum(
                            jnp.where(ok, 0.0, 1.0), jnp.maximum(bad_o[0:8], bad_o[8:16])))
        return [functools.partial(item, i) for i in range(na_items)]

    def body(sb_list, sa_list, carry, fill=()):
        box = dict(mem=carry[0], bad=carry[1])
        bs = [it for sb in sb_list for it in b_stream(sb, box)]
        as_ = [it for sa in sa_list for it in a_stream(sa, box)]
        if bs and as_:
            _interleave(bs, as_)
        else:
            _interleave(bs or as_, list(fill))
        return box["mem"], box["bad"]

    carry = (mem_ref[...].astype(F32), jnp.zeros((8, 128), F32))

    first_left = NQ - rlag
    _dma_block(1, lambda _: cp_wob.start(priority=1))
    n_left = NW - first_left
    for t in range(npre):
        lo_, hi_ = first_left + t * n_left // npre, first_left + (t + 1) * n_left // npre
        _dma_block(hi_ - lo_, lambda k, lo_=lo_: wait_w(lo_ + k))
        carry = body([], [t], carry, [f for j in range(lo_, hi_) for f in relay_pieces(j)])
    _dma_block(1, lambda _: cp_wob.wait())
    cp_woa.start(priority=1)

    n_main = (NSEG - npre) // un

    def step_u(t, c):
        return body([t * un + u for u in range(un)], [t * un + u + npre for u in range(un)], c)

    carry = lax.fori_loop(0, n_main, step_u, carry)

    @pl.when(jnp.max(carry[1]) > 0.0)
    def _():
        row_head = lax.broadcasted_iota(jnp.int32, (128, 128), 0) // DHA
        ck = 256

        def safe_block(i, c):
            hh, qt = i // NQ, i % NQ
            g = hh // 8
            qcols = _ds(qt * 128, 128)
            qv = _unpack(qt_u[_ds(g * 64, 64), qcols])
            qm = jnp.where(row_head == hh % 8, qv, jnp.zeros_like(qv))

            def scores(ch):
                return _nn(_unpack(k_u[g, _ds(ch * (ck // 2), ck // 2), :]), qm)

            def pass1(ch, m):
                return jnp.maximum(m, jnp.max(scores(ch), axis=0, keepdims=True))
            m = lax.fori_loop(0, S // ck, pass1, jnp.full((1, 128), -jnp.inf, F32))

            def pass2(ch, acc):
                o, l = acc
                p = jnp.exp2(scores(ch) - m)
                vt = _unpack(vt_u[_ds(hh * 8, 8), _ds(ch * ck, ck)])
                return o + _nn(vt, p.astype(BF)), l + jnp.sum(p, axis=0, keepdims=True)
            o, l = lax.fori_loop(0, S // ck, pass2, (jnp.zeros((DHA, 128), F32), jnp.zeros((1, 128), F32)))
            ot_s[_ds(hh * DHA, DHA), qcols] = (o * (1.0 / l)).astype(BF)
            return c
        lax.fori_loop(0, HA * NQ, safe_block, 0)

    cp_woa.wait()

    def final_tile(t):
        rows = _ds(t * 128, 128)
        a = _nn(ot_s[:, rows].T, woa_v[...])
        gq = g_s[rows, :]
        gq4 = jnp.concatenate([gq] * (D // 128), axis=1)
        out_v[rows, :] = (gq4 * a + b_s[rows, :]).astype(BF)

    ready = (NSEG - npre) * SEG // 128
    split = [0, FSPLIT, ready]
    for k in range(npre):
        tiles = range(split[k], split[k + 1])
        carry = body([NSEG - npre + k], [], carry, [functools.partial(final_tile, t) for t in tiles])
        _dma_block(len(tiles), lambda j, k=k: cp_out(split[k] + j).start())
    for t in range(ready, NQ):
        final_tile(t)
    _dma_block(NQ - ready, lambda j: cp_out(ready + j).start())

    def drain(t, c):
        cp_out(t).wait()
        return c
    lax.fori_loop(0, NQ, drain, 0)


@jax.jit
def _impl(A_x, A_wqkv, A_wo, B_mem0, B_Wq, B_Wk, B_Wv, B_Wo, gate_w):
    any_spec = pl.BlockSpec(memory_space=pl.ANY)
    vmem_spec = pl.BlockSpec(memory_space=pltpu.VMEM)
    out = pl.pallas_call(
        _kernel,
        out_shape=jax.ShapeDtypeStruct((S, D), BF),
        in_specs=[any_spec] * 7 + [vmem_spec, vmem_spec],
        out_specs=any_spec,
        scratch_shapes=[
            pltpu.VMEM((S, D), BF),
            pltpu.VMEM((D, 3 * D), BF),
            pltpu.VMEM((D, D), BF),
            pltpu.VMEM((3, D * HB, DHB), BF),
            pltpu.VMEM((HB * DHB, D), BF),
            pltpu.VMEM((S // 2, D), U32),
            pltpu.VMEM((2, D // 2, D), U32),
            pltpu.VMEM((D // 2, D), U32),
            pltpu.VMEM((HB, D // 2, 3 * DHB), U32),
            pltpu.VMEM((D // 2, S), U32),
            pltpu.VMEM((4, S // 2, 128), U32),
            pltpu.VMEM((D // 2, S), U32),
            pltpu.VMEM((D, S), BF),
            pltpu.VMEM((S, D), F32),
            pltpu.VMEM((S, 128), F32),
            pltpu.VMEM((S, D), BF),
            pltpu.VMEM((WO_DEFER, L, DHB), F32),
            pltpu.SemaphoreType.DMA((3,)),
            pltpu.SemaphoreType.DMA((4,)),
            pltpu.SemaphoreType.DMA((3 * NW,)),
            pltpu.SemaphoreType.DMA((NQ,)),
        ],
        compiler_params=pltpu.CompilerParams(vmem_limit_bytes=100 * 2 ** 20),
        name="gated_mix_kernel",
    )(A_x.reshape(S, D), A_wqkv, A_wo,
      B_Wq.reshape(D * HB, DHB), B_Wk.reshape(D * HB, DHB), B_Wv.reshape(D * HB, DHB),
      B_Wo.reshape(HB * DHB, D), B_mem0.reshape(M, D), gate_w)
    return out.reshape(1, S, D)


def pallas_gated_mix__mha_block__memory_aug_recurrent_mem_tr__prompt_kernel(
    A_x, A_wqkv, A_wo, B_x, B_mem0, B_Wq, B_Wk, B_Wv, B_Wo, B_seg_len, gate_w,
):
    del B_x
    if isinstance(B_seg_len, int):
        assert B_seg_len == SEG, "the kernel is specialised to seg_len == 32"
    return _impl(A_x, A_wqkv, A_wo, B_mem0, B_Wq, B_Wk, B_Wv, B_Wo, gate_w)
```
